```python
import os as _os
_os.environ.setdefault("JAX_PLATFORMS", "cpu")
import jax
import jax.numpy as jnp

def _softmax(x, axis=-1):
    return jax.nn.softmax(x, axis=axis)
def _gelu(x):
    return jax.nn.gelu(x, approximate=True)
def _silu(x):
    return jax.nn.silu(x)
def _sigmoid(x):
    return jax.nn.sigmoid(x)
def _layernorm(x, axis=-1, eps=1e-5):
    m = jnp.mean(x, axis=axis, keepdims=True)
    v = jnp.var(x, axis=axis, keepdims=True)
    return (x - m) / jnp.sqrt(v + eps)
def _scatter_add(tgt, idx, src, axis=0):
    return tgt.at[idx].add(src)
def _segment_sum(src, seg, n):
    return jax.ops.segment_sum(src, seg, n)
class _Rng:
    def __init__(self, key):
        self._k = key
    def _next(self):
        self._k, sub = jax.random.split(self._k)
        return sub
    def normal(self, shape):
        return jax.random.normal(self._next(), shape, dtype=jnp.bfloat16)
    def randint(self, lo, hi, shape):
        return jax.random.randint(self._next(), shape, lo, hi, dtype=jnp.int32)
    def uniform(self, shape, lo=0.0, hi=1.0):
        return jax.random.uniform(self._next(), shape, jnp.bfloat16, lo, hi)
    def permutation(self, n):
        return jax.random.permutation(self._next(), n)


kernel_name = 'sequential_preLN__linear_kernel_hedgehog__glu_gated_swiglu__prompt'

def setup_inputs():
    _rng = _Rng(jax.random.key(int.from_bytes(__import__("os").urandom(4), "little")))
    _w = (lambda a: (lambda t: t.astype(jnp.bfloat16) if jnp.issubdtype(t.dtype, jnp.floating) else t)(jnp.asarray(a)))
    def _A_setup():
        B, S, D, H = 1, 2048, 640, 32
        Dh = D // H
        return {
            "x": _w((lambda *s: _rng.normal(s) * 0.05)(B, S, D)),
            "wqkv": _w((lambda *s: _rng.normal(s) * 0.2)(D, 3 * D)),
            "w_phi": _w((lambda *s: _rng.normal(s) * 0.2)(H, Dh, Dh) * (Dh ** -0.5)),
            "wo": _w((lambda *s: _rng.normal(s) * 0.05)(D, D)),
        }
    _A_in = _A_setup()

    def _B_setup():
        B, S, D, F = 1, 2048, 640, 1536
        return {
            "x": _w((lambda *s: _rng.normal(s) * 0.05)(B, S, D)),
            "w1": _w((lambda *s: _rng.normal(s) * 0.05)(D, F) * (2.0 / D) ** 0.5),
            "w3": _w((lambda *s: _rng.normal(s) * 0.05)(D, F) * (2.0 / D) ** 0.5),
            "w2": _w((lambda *s: _rng.normal(s) * 0.05)(F, D) * (2.0 / F) ** 0.5),
        }
    _B_in = _B_setup()

    return {
        "A_x": _A_in["x"],
        "A_wqkv": _A_in["wqkv"],
        "A_w_phi": _A_in["w_phi"],
        "A_wo": _A_in["wo"],
        "B_x": _B_in["x"],
        "B_w1": _B_in["w1"],
        "B_w3": _B_in["w3"],
        "B_w2": _B_in["w2"],
    }

def reference(A_x, A_wqkv, A_w_phi, A_wo, B_x, B_w1, B_w3, B_w2):
    def _A_ref(x, wqkv, w_phi, wo):
        B, S, D = x.shape
        H = 32; Dh = D // H
        qkv = (lambda x, *d: x.transpose(*d))((x @ wqkv).reshape(B, S, 3, H, Dh), 2, 0, 3, 1, 4)
        q, k, v = qkv[0], qkv[1], qkv[2]
        pq = jnp.einsum("bhsd,hdf->bhsf", q, w_phi)
        pk = jnp.einsum("bhsd,hdf->bhsf", k, w_phi)
        phi_q = jnp.concatenate([_softmax(pq, axis=-1), _softmax(-pq, axis=-1)], axis=-1)
        phi_k = jnp.concatenate([_softmax(pk, axis=-1), _softmax(-pk, axis=-1)], axis=-1)
        kv = jnp.einsum("bhsf,bhsd->bhfd", phi_k, v)
        z  = jnp.einsum("bhsf->bhf", phi_k)
        num = jnp.einsum("bhqf,bhfd->bhqd", phi_q, kv)
        den = jnp.einsum("bhqf,bhf->bhq", phi_q, z)[..., None] + 1e-6
        o = num / den
        return (lambda x, *d: x.transpose(*d))(o, 0, 2, 1, 3).reshape(B, S, D) @ wo

    def _B_ref(x, w1, w3, w2):
        gate = jnp.einsum("bsd,df->bsf", x, w1)
        up = jnp.einsum("bsd,df->bsf", x, w3)
        h = _silu(gate) * up
        out = jnp.einsum("bsf,fd->bsd", h, w2)
        return out

    x = A_x
    h = x + _A_ref(_layernorm(x, axis=-1), A_wqkv, A_w_phi, A_wo)
    h2 = h + _B_ref(_layernorm(h, axis=-1), B_w1, B_w3, B_w2)
    return h2
```

```python
import functools
import jax
import jax.numpy as jnp
from jax import lax
import jax.experimental.pallas as pl
import jax.experimental.pallas.tpu as pltpu

S, D, H, DH, F = 2048, 640, 32, 20, 1536
NP = H // 2
PR = 2 * DH
NT_DIMS = (((1,), (1,)), ((), ()))
BF = jnp.bfloat16
F32 = jnp.float32
EPS = 1e-5
LOG2E = 1.4426950408889634


def _rcp(x):
    r = pl.reciprocal(x, approx=True)
    return r * (2.0 - x * r)


def _ln(x):
    m = jnp.mean(x, axis=-1, keepdims=True)
    xc = x - m
    v = jnp.mean(xc * xc, axis=-1, keepdims=True)
    return xc * lax.rsqrt(v + EPS)


def _red(x3, op):
    r = op(op(op(x3[0], x3[1]), op(x3[2], x3[3])), x3[4])
    r = op(r, pltpu.roll(r, 2, 0))
    r = op(r, pltpu.roll(r, 4, 0))
    return r


def _feat(p, T):
    p3 = p.reshape(5, 8, T)
    mx = _red(p3, jnp.maximum)
    mn = _red(p3, jnp.minimum)
    ep = jnp.exp2(p3 - mx[None])
    en = jnp.exp2(mn[None] - p3)
    rp = _rcp(_red(ep, jnp.add))
    rn = _rcp(_red(en, jnp.add))
    phi = jnp.concatenate([ep * rp[None], en * rn[None]], axis=0)
    return phi.reshape(2 * PR, T).astype(BF)


def _kernel(x_hbm, wqkv_hbm, wphi_hbm, wo_hbm, w1_hbm, w3_hbm, w2_hbm, out_hbm,
            x_v, out_v, xn_v, wphi_v, wqkv_v, wo_v, w1_v, w3_v, w2_v, wt_v, wp_v, phiq_v, kv_acc, kvb_v,
            sems, xsems, osems, *, TA, TB, SB, FC):
    NA = S // TA
    NB = S // TB

    def wcopy(s):
        return pltpu.make_async_copy(wqkv_hbm.at[:, pl.ds(D * s, D)], wqkv_v.at[:, pl.ds(D * s, D)], sems.at[s])

    def xcopy(i):
        return pltpu.make_async_copy(x_hbm.at[pl.ds(i * TA, TA)], x_v.at[pl.ds(i * TA, TA)], xsems.at[i])

    def ocopy(j):
        return pltpu.make_async_copy(out_v.at[pl.ds(j * SB, SB)], out_hbm.at[pl.ds(j * SB, SB)], osems.at[j])

    cp_phi = pltpu.make_async_copy(wphi_hbm, wphi_v, sems.at[3])
    cp_wo = pltpu.make_async_copy(wo_hbm, wo_v, sems.at[4])
    cp_w1 = pltpu.make_async_copy(w1_hbm, w1_v, sems.at[5])
    cp_w3 = pltpu.make_async_copy(w3_hbm, w3_v, sems.at[6])
    cp_w2 = pltpu.make_async_copy(w2_hbm, w2_v, sems.at[7])

    with jax.named_scope("prologue"):
        cp_phi.start()
        wcopy(1).start(); wcopy(0).start(); xcopy(0).start(); wcopy(2).start()
        for i in range(1, NA):
            xcopy(i).start()
        cp_wo.start(); cp_w1.start(); cp_w3.start(); cp_w2.start()

        kv_acc[...] = jnp.zeros_like(kv_acc)
        wp_v[...] = jnp.zeros_like(wp_v)
        yh = lax.broadcasted_iota(jnp.int32, (H, D), 0)
        yc = lax.broadcasted_iota(jnp.int32, (H, D), 1)
        Y = jnp.where(yc // DH == yh, 1.0, 0.0).astype(BF)
        cmod = lax.broadcasted_iota(jnp.int32, (24, D), 1) % DH
        er = lax.broadcasted_iota(jnp.int32, (PR, 24), 0)
        ec = lax.broadcasted_iota(jnp.int32, (PR, 24), 1)
        E = jnp.where(er // 2 == ec, 1.0, 0.0).astype(BF)
        rr = lax.broadcasted_iota(jnp.int32, (4 * PR, 128), 0)
        cc = lax.broadcasted_iota(jnp.int32, (4 * PR, 128), 1)
        cp_phi.wait()
        wp_v[:, pl.ds(0, DH), :] = wphi_v[...].astype(F32)
        V = wp_v[...].reshape(DH * 24, H).astype(BF)
        C = jnp.dot(V, Y, preferred_element_type=F32).reshape(DH, 24, D)
        B = jnp.zeros((24, D), F32)
        for d in range(DH):
            B = jnp.where(cmod == d, C[d], B)
        B2 = jnp.dot(E, B.astype(BF), preferred_element_type=F32)
        As = []
        for t in range(5):
            b2 = B2[:, 128 * t:128 * (t + 1)]
            a = jnp.concatenate([b2, b2, b2, b2], axis=0)
            head_r = 2 * (3 * t + rr // PR) + rr % 2
            As.append(jnp.where((cc + 128 * t) // DH == head_r, a, 0.0).astype(BF))
        for s in (1, 0):
            wcopy(s).wait()
            prev = None
            for t in range(5):
                w = wqkv_v[:, pl.ds(D * s + 128 * t, 128)]
                res = lax.dot_general(As[t], w, NT_DIMS, preferred_element_type=F32)
                if prev is not None:
                    res = jnp.concatenate([res[:PR] + prev, res[PR:]], axis=0)
                n = 160 if t == 4 else 120
                wt_v[pl.ds(D * s + 120 * t, n), :] = (res[:n] * LOG2E).astype(BF)
                prev = res[120:]
        xcopy(0).wait()
        xn_v[0] = _ln(x_v[pl.ds(0, TA), :].astype(F32)).astype(BF)
        wcopy(2).wait()
        wt_v[pl.ds(2 * D, D), :] = wqkv_v[:, pl.ds(2 * D, D)].astype(F32).T.astype(BF)

    def body_a(i, carry):
        @pl.when(i + 1 < NA)
        def _():
            xcopy(i + 1).wait()

        slot = i % 2
        xn = xn_v[slot]
        col = pl.multiple_of(i * TA, TA)
        pk = lax.dot_general(wt_v[pl.ds(D, D), :], xn, NT_DIMS, preferred_element_type=F32)
        pv = lax.dot_general(wt_v[pl.ds(2 * D, D), :], xn, NT_DIMS, preferred_element_type=F32)
        pq = lax.dot_general(wt_v[pl.ds(0, D), :], xn, NT_DIMS, preferred_element_type=F32)
        ones = jnp.ones((8, TA), F32)
        for p in range(NP):
            phik = _feat(pk[PR * p:PR * (p + 1)], TA)
            vt = jnp.concatenate([pv[PR * p:PR * (p + 1)], ones], axis=0).astype(BF)
            kv_acc[p] += lax.dot_general(vt, phik, NT_DIMS, preferred_element_type=F32)
        for p in range(NP):
            phiq_v[pl.ds(2 * PR * p, 2 * PR), pl.ds(col, TA)] = _feat(pq[PR * p:PR * (p + 1)], TA)
        nxt = pl.multiple_of(jnp.minimum(i + 1, NA - 1) * TA, TA)
        xn_v[1 - slot] = _ln(x_v[pl.ds(nxt, TA), :].astype(F32)).astype(BF)
        return carry

    with jax.named_scope("phaseA"):
        lax.fori_loop(0, NA, body_a, 0)

    with jax.named_scope("fin"):
        rr = lax.broadcasted_iota(jnp.int32, (48, 2 * PR), 0)
        cc = lax.broadcasted_iota(jnp.int32, (48, 2 * PR), 1)
        head_r = jnp.where(rr < PR, rr // DH, (rr - PR) // 4)
        mask = head_r == cc % 2
        for p in range(NP):
            kvb_v[p] = jnp.where(mask, kv_acc[p], 0.0).astype(BF)
        cp_wo.wait(); cp_w1.wait(); cp_w3.wait(); cp_w2.wait()

    def attn(row):
        sub = lax.broadcasted_iota(jnp.int32, (8, SB), 0)
        ots = []
        for p in range(NP):
            nd = jnp.dot(kvb_v[p], phiq_v[pl.ds(2 * PR * p, 2 * PR), pl.ds(row, SB)],
                         preferred_element_type=F32)
            r = _rcp(nd[PR:PR + 8] + 1e-6)
            rs = pltpu.roll(r, 4, 0)
            ra = jnp.where(sub < 4, r, rs)
            rb = jnp.where(sub < 4, rs, r)
            ots.append(nd[:PR] * jnp.concatenate([ra, ra, r, rb, rb], axis=0))
        o = jnp.concatenate(ots, axis=0).T.astype(BF)
        h = x_v[pl.ds(row, SB), :].astype(F32) + jnp.dot(o, wo_v[...], preferred_element_type=F32)
        return h, _ln(h).astype(BF)

    def ffn(h, hn):
        acc = h
        for c in range(F // FC):
            gate = jnp.dot(hn, w1_v[:, pl.ds(FC * c, FC)], preferred_element_type=F32)
            up = jnp.dot(hn, w3_v[:, pl.ds(FC * c, FC)], preferred_element_type=F32)
            act = (gate * _rcp(1.0 + jnp.exp(-gate)) * up).astype(BF)
            acc = acc + jnp.dot(act, w2_v[pl.ds(FC * c, FC), :], preferred_element_type=F32)
        return acc.astype(BF)

    def body_b(j, carry):
        nsub = TB // SB
        rows = [pl.multiple_of(j * TB + s * SB, SB) for s in range(nsub)]
        hs = [attn(r) for r in rows]
        for s in range(nsub):
            out_v[pl.ds(rows[s], SB), :] = ffn(*hs[s])
            ocopy(j * nsub + s).start()
        return carry

    with jax.named_scope("phaseB"):
        lax.fori_loop(0, NB, body_b, 0)

    with jax.named_scope("tail"):
        for j in range(S // SB):
            ocopy(j).wait()


def build(A_x, A_wqkv, A_w_phi, A_wo, B_x, B_w1, B_w3, B_w2, TA=512, TB=512, SB=256, FC=512):
    x2 = A_x.reshape(S, D)
    wphi_t = A_w_phi.transpose(1, 2, 0)
    any_spec = pl.BlockSpec(memory_space=pl.ANY)
    out = pl.pallas_call(
        functools.partial(_kernel, TA=TA, TB=TB, SB=SB, FC=FC),
        in_specs=[any_spec] * 7,
        out_specs=any_spec,
        out_shape=jax.ShapeDtypeStruct((S, D), BF),
        scratch_shapes=[
            pltpu.VMEM((S, D), BF),
            pltpu.VMEM((S, D), BF),
            pltpu.VMEM((2, TA, D), BF),
            pltpu.VMEM((DH, DH, H), BF),
            pltpu.VMEM((D, 3 * D), BF),
            pltpu.VMEM((D, D), BF),
            pltpu.VMEM((D, F), BF),
            pltpu.VMEM((D, F), BF),
            pltpu.VMEM((F, D), BF),
            pltpu.VMEM((3 * D, D), BF),
            pltpu.VMEM((DH, 24, H), F32),
            pltpu.VMEM((2 * D, S), BF),
            pltpu.VMEM((NP, 48, 2 * PR), F32),
            pltpu.VMEM((NP, 48, 2 * PR), BF),
            pltpu.SemaphoreType.DMA((8,)),
            pltpu.SemaphoreType.DMA((S // TA,)),
            pltpu.SemaphoreType.DMA((S // SB,)),
        ],
        compiler_params=pltpu.CompilerParams(
            vmem_limit_bytes=100 * 1024 * 1024,
        ),
    )(x2, A_wqkv, wphi_t, A_wo, B_w1, B_w3, B_w2)
    return out.reshape(1, S, D)


@jax.jit
def pallas_sequential_preLN__linear_kernel_hedgehog__glu_gated_swiglu__prompt_kernel(
        A_x, A_wqkv, A_w_phi, A_wo, B_x, B_w1, B_w3, B_w2):
    return build(A_x, A_wqkv, A_w_phi, A_wo, B_x, B_w1, B_w3, B_w2)
```

```python
import functools
import math
import jax
import jax.numpy as jnp
from jax import lax
import jax.experimental.pallas as pl
import jax.experimental.pallas.tpu as pltpu

S, D, H, DH, F = 2048, 640, 32, 20, 1536
NP = H // 2
PR = 2 * DH
NT_DIMS = (((1,), (1,)), ((), ()))
BF = jnp.bfloat16
F32 = jnp.float32
EPS = 1e-5
LOG2E = 1.4426950408889634


def _rcp(x):
    r = pl.reciprocal(x, approx=True)
    return r * (2.0 - x * r)


def _ln(x):
    m = jnp.mean(x, axis=-1, keepdims=True)
    xc = x - m
    v = jnp.mean(xc * xc, axis=-1, keepdims=True)
    return xc * lax.rsqrt(v + EPS)


def _red(x3, op):
    r = op(op(op(x3[0], x3[1]), op(x3[2], x3[3])), x3[4])
    r = op(r, pltpu.roll(r, 2, 0))
    r = op(r, pltpu.roll(r, 4, 0))
    return r


def _feat(p, T):
    p3 = p.reshape(5, 8, T)
    mx = _red(p3, jnp.maximum)
    mn = _red(p3, jnp.minimum)
    ep = jnp.exp2(p3 - mx[None])
    en = jnp.exp2(mn[None] - p3)
    rp = _rcp(_red(ep, jnp.add))
    rn = _rcp(_red(en, jnp.add))
    phi = jnp.concatenate([ep * rp[None], en * rn[None]], axis=0)
    return phi.reshape(2 * PR, T).astype(BF)


def _kernel(x_hbm, wqkv_hbm, wphi_hbm, wo_hbm, w1_hbm, w3_hbm, w2_hbm, out_hbm,
            x_v, out_v, xn_v, vt_v, wphi_v, wqkv_v, wo_v, w1_v, w3_v, w2_v, wt_v, wp_v, y_v, phiq_v, kv_acc, kvb_v,
            sems, *, TA, TB, SB, FC, XA, OSPLIT):
    NA = S // TA
    NB = S // TB

    def wcopy(c0, n, sem):
        return pltpu.make_async_copy(wqkv_hbm.at[:, pl.ds(c0, n)], wqkv_v.at[:, pl.ds(c0, n)], sems.at[sem])

    def xcopy(i):
        return pltpu.make_async_copy(x_hbm.at[pl.ds(i * TA, TA)], x_v.at[pl.ds(i * TA, TA)], sems.at[min(i - 1, 1)])

    def ocopy(r, n):
        return pltpu.make_async_copy(out_v.at[pl.ds(r, n)], out_hbm.at[pl.ds(r, n)], sems.at[3])

    cp_q = wcopy(0, D, 4)
    cp_k = wcopy(D, D, 3)
    cp_va1 = wcopy(2 * D + 512, 128, 5)
    cp_va2 = wcopy(2 * D + 256, 256, 1)
    cp_vb = wcopy(2 * D, 256, 2)
    cp_xa = pltpu.make_async_copy(x_hbm.at[pl.ds(0, XA)], x_v.at[pl.ds(0, XA)], sems.at[0])
    cp_xb = pltpu.make_async_copy(x_hbm.at[pl.ds(XA, TA - XA)], x_v.at[pl.ds(XA, TA - XA)], sems.at[2])
    cp_phi = pltpu.make_async_copy(wphi_hbm, wphi_v, sems.at[2])
    cp_wo = pltpu.make_async_copy(wo_hbm, wo_v, sems.at[2])
    cp_w1 = pltpu.make_async_copy(w1_hbm, w1_v, sems.at[2])
    cp_w3 = pltpu.make_async_copy(w3_hbm, w3_v, sems.at[2])
    cp_w2 = pltpu.make_async_copy(w2_hbm, w2_v, sems.at[2])

    def proj(s, xn):
        return lax.dot_general(wt_v[pl.ds(D * s, D), :], xn, NT_DIMS, preferred_element_type=F32)

    def dot2(w, xn):
        tiles = (xn.shape[0] // 128) * (xn.shape[1] // 128)
        ns = 2 if tiles == 5 and w.shape[1] == 128 else 4 // math.gcd(4, tiles)
        m = w.shape[0] // ns
        return jnp.concatenate([lax.dot_general(w[m * u:m * (u + 1)], xn, NT_DIMS, preferred_element_type=F32)
                                for u in range(ns)], axis=0)

    def vstore(pv, p0, c0, n):
        ones = jnp.ones((8, n), F32)
        for p in range(pv.shape[0] // PR):
            vt_v[p0 + p, :, pl.ds(c0, n)] = jnp.concatenate([pv[PR * p:PR * (p + 1)], ones], axis=0).astype(BF)

    def vproj(xn):
        vstore(proj(2, xn), 0, 0, TA)

    def vrows(r0, n, xn):
        return lax.dot_general(wt_v[pl.ds(2 * D + r0, n), :], xn, NT_DIMS, preferred_element_type=F32)

    def transpose_v(c0, n):
        wt_v[pl.ds(2 * D + c0, n), :] = wqkv_v[:, pl.ds(2 * D + c0, n)].astype(F32).T.astype(BF)

    def fold(As, s):
        prev = None
        for t in range(5):
            w = wqkv_v[:, pl.ds(D * s + 128 * t, 128)]
            res = dot2(As[t], w)
            if prev is not None:
                res = jnp.concatenate([res[:PR] + prev, res[PR:]], axis=0)
            n = 160 if t == 4 else 120
            wt_v[pl.ds(D * s + 120 * t, n), :] = (res[:n] * LOG2E).astype(BF)
            prev = res[120:]

    def kstep(xn):
        pk = proj(1, xn)
        return [_feat(pk[PR * p:PR * (p + 1)], TA) for p in range(NP)]

    def qstep(xn, col):
        pq = proj(0, xn)
        for p in range(NP):
            phiq_v[pl.ds(2 * PR * p, 2 * PR), pl.ds(col, TA)] = _feat(pq[PR * p:PR * (p + 1)], TA)

    def astep(vts, phiks, first=False, last=False):
        if last:
            rr = lax.broadcasted_iota(jnp.int32, (48, 2 * PR), 0)
            cc = lax.broadcasted_iota(jnp.int32, (48, 2 * PR), 1)
            head_r = jnp.where(rr < PR, rr // DH, (rr - PR) // 4)
            mask = head_r == cc % 2
        for p in range(NP):
            kv = lax.dot_general(vts[p], phiks[p], NT_DIMS, preferred_element_type=F32)
            if not first:
                kv = kv + kv_acc[p]
            if last:
                kvb_v[p] = jnp.where(mask, kv, 0.0).astype(BF)
            else:
                kv_acc[p] = kv

    def vstep(row):
        xn1 = _ln(x_v[pl.ds(row, TA), :].astype(F32)).astype(BF)
        xn_v[...] = xn1
        vproj(xn1)

    with jax.named_scope("prologue"):
        cp_xa.start(); cp_va1.start(); cp_va2.start(); cp_xb.start(); cp_vb.start(); cp_phi.start()
        cp_k.start(); cp_q.start()

        c8 = lax.broadcasted_iota(jnp.int32, (8, D), 1)
        r8 = lax.broadcasted_iota(jnp.int32, (8, D), 0)
        ch = c8 // DH
        cd = c8 - ch * DH
        key = ch + H * (cd % 4) - r8
        Y = jnp.concatenate([jnp.where(key == 8 * j, 1.0, 0.0) for j in range(16)], axis=0).astype(BF)
        cg = cd // 4
        hp = ch - r8 % 2
        y_v[...] = Y
        with jax.named_scope("w_xa"):
            cp_xa.wait()
        xcopy(1).start()
        xna = _ln(x_v[pl.ds(0, XA), :].astype(F32)).astype(BF)
        xn_v[pl.ds(0, XA), :] = xna
        with jax.named_scope("w_va1"):
            cp_va1.wait()
        transpose_v(512, 128)
        with jax.named_scope("w_va2"):
            cp_va2.wait()
        for i in range(2, NA):
            xcopy(i).start()
        transpose_v(384, 128)
        transpose_v(256, 128)
        for g in (7, 6, 5, 4):
            vstore(vrows(80 * g, 80, xna), 2 * g, 0, XA)
        with jax.named_scope("w_b"):
            cp_xb.wait(); cp_vb.wait(); cp_phi.wait()
        cp_wo.start(); cp_w1.start(); cp_w3.start(); cp_w2.start()
        p3 = vrows(256, 64, xna)
        w = wphi_v[...].astype(F32)
        for g in range(5):
            vk = jnp.concatenate([w[4 * g + l] for l in range(4)], axis=1)
            wp_v[g, pl.ds(0, DH, stride=2), :] = vk
            wp_v[g, pl.ds(1, DH, stride=2), :] = vk
        C = jnp.dot(wp_v[...].reshape(5 * PR, 128).astype(BF), y_v[...], preferred_element_type=F32)
        transpose_v(128, 128)
        transpose_v(0, 128)
        vstore(jnp.concatenate([vrows(160, 96, xna), p3], axis=0), 4, 0, XA)
        vstore(vrows(80, 80, xna), 2, 0, XA)
        vstore(vrows(0, 80, xna), 0, 0, XA)
        xnb = _ln(x_v[pl.ds(XA, TA - XA), :].astype(F32)).astype(BF)
        xn_v[pl.ds(XA, TA - XA), :] = xnb
        vstore(dot2(wt_v[pl.ds(2 * D, D), :], xnb), 0, XA, TA - XA)
        C = C.reshape(5, 5, 8, D)
        B2 = C[0]
        for g in range(1, 5):
            B2 = jnp.where((cg == g)[None], C[g], B2)
        As = []
        for t in range(5):
            b2 = B2[:, :, 128 * t:128 * (t + 1)]
            hpt = hp[:, 128 * t:128 * (t + 1)]
            a = jnp.concatenate([jnp.where((hpt == 2 * (3 * t + u))[None], b2, 0.0) for u in range(4)], axis=0)
            As.append(a.reshape(4 * PR, 128).astype(BF))
        with jax.named_scope("w_k"):
            cp_k.wait()
        fold(As, 1)
        phiks0 = kstep(xn_v[...])
        with jax.named_scope("w_q"):
            cp_q.wait(); xcopy(1).wait()
        fold(As, 0)
        qstep(xn_v[...], 0)
        astep([vt_v[p] for p in range(NP)], phiks0, first=True)
        vstep(TA)

    def body_a(i, carry, last=False):
        if not last:
            @pl.when(i == 1)
            def _():
                for t in range(2, NA):
                    xcopy(t).wait()

            @pl.when(i == NA - 2)
            def _():
                cp_wo.wait(); cp_w1.wait(); cp_w3.wait(); cp_w2.wait()
        xn = xn_v[...]
        vts = [vt_v[p] for p in range(NP)]
        qstep(xn, i * TA if last else pl.multiple_of(i * TA, TA))
        phiks = kstep(xn)
        astep(vts, phiks, last=last)
        if not last:
            vstep(pl.multiple_of((i + 1) * TA, TA))
        return carry

    with jax.named_scope("phaseA"):
        lax.fori_loop(1, NA - 1, body_a, 0)
        body_a(NA - 1, 0, last=True)

    def attn(row):
        sub = lax.broadcasted_iota(jnp.int32, (8, SB), 0)
        ots = []
        for p in range(NP):
            nd = jnp.dot(kvb_v[p], phiq_v[pl.ds(2 * PR * p, 2 * PR), pl.ds(row, SB)],
                         preferred_element_type=F32)
            r = _rcp(nd[PR:PR + 8] + 1e-6)
            rs = pltpu.roll(r, 4, 0)
            ra = jnp.where(sub < 4, r, rs)
            rb = jnp.where(sub < 4, rs, r)
            ots.append(nd[:PR] * jnp.concatenate([ra, ra, r, rb, rb], axis=0))
        return jnp.concatenate(ots, axis=0).T.astype(BF)

    def oproj(row, o):
        h = x_v[pl.ds(row, SB), :].astype(F32) + jnp.dot(o, wo_v[...], preferred_element_type=F32)
        return h, _ln(h).astype(BF)

    def ffn(h, hn, row, splits):
        acc = h
        nc = F // FC
        for c in range(nc):
            gate = jnp.dot(hn, w1_v[:, pl.ds(FC * c, FC)], preferred_element_type=F32)
            up = jnp.dot(hn, w3_v[:, pl.ds(FC * c, FC)], preferred_element_type=F32)
            hg = 0.5 * gate
            act = ((hg + hg * jnp.tanh(hg)) * up).astype(BF)
            if c + 1 < nc:
                acc = acc + jnp.dot(act, w2_v[pl.ds(FC * c, FC), :], preferred_element_type=F32)
        r0 = 0
        for n in splits:
            res = acc[r0:r0 + n] + jnp.dot(act[r0:r0 + n], w2_v[pl.ds(F - FC, FC), :], preferred_element_type=F32)
            rw = pl.multiple_of(row + r0, 64)
            out_v[pl.ds(rw, n), :] = res.astype(BF)
            ocopy(rw, n).start()
            r0 += n

    nsub = TB // SB
    splits = [(SB,)] * (nsub - 1) + [OSPLIT]

    def body_b(j, carry):
        rows = [pl.multiple_of(j * TB + s * SB, SB) for s in range(nsub)]
        os_ = [attn(r) for r in rows]
        hs = [oproj(r, o) for r, o in zip(rows, os_)]
        for s in range(nsub):
            ffn(*hs[s], rows[s], splits[s])
        return carry

    with jax.named_scope("phaseB"):
        lax.fori_loop(0, NB, body_b, 0)

    with jax.named_scope("tail"):
        for j in range(NB):
            r0 = j * TB
            for sp in splits:
                for n in sp:
                    ocopy(r0, n).wait()
                    r0 += n


def build(A_x, A_wqkv, A_w_phi, A_wo, B_x, B_w1, B_w3, B_w2, TA=512, TB=512, SB=256, FC=512, XA=384, OS=2):
    OSPLIT = {0: (256,), 1: (128, 128), 2: (128, 64, 64), 3: (192, 64)}[OS]
    x2 = A_x.reshape(S, D)
    wphi_t = A_w_phi.transpose(1, 2, 0)
    any_spec = pl.BlockSpec(memory_space=pl.ANY)
    out = pl.pallas_call(
        functools.partial(_kernel, TA=TA, TB=TB, SB=SB, FC=FC, XA=XA, OSPLIT=OSPLIT),
        in_specs=[any_spec] * 7,
        out_specs=any_spec,
        out_shape=jax.ShapeDtypeStruct((S, D), BF),
        scratch_shapes=[
            pltpu.VMEM((S, D), BF),
            pltpu.VMEM((S, D), BF),
            pltpu.VMEM((TA, D), BF),
            pltpu.VMEM((NP, 48, TA), BF),
            pltpu.VMEM((DH, DH, H), BF),
            pltpu.VMEM((D, 3 * D), BF),
            pltpu.VMEM((D, D), BF),
            pltpu.VMEM((D, F), BF),
            pltpu.VMEM((D, F), BF),
            pltpu.VMEM((F, D), BF),
            pltpu.VMEM((3 * D, D), BF),
            pltpu.VMEM((5, PR, 128), F32),
            pltpu.VMEM((128, D), BF),
            pltpu.VMEM((2 * D, S), BF),
            pltpu.VMEM((NP, 48, 2 * PR), F32),
            pltpu.VMEM((NP, 48, 2 * PR), BF),
            pltpu.SemaphoreType.DMA((6,)),
        ],
        compiler_params=pltpu.CompilerParams(
            vmem_limit_bytes=100 * 1024 * 1024,
        ),
    )(x2, A_wqkv, wphi_t, A_wo, B_w1, B_w3, B_w2)
    return out.reshape(1, S, D)


@jax.jit
def pallas_sequential_preLN__linear_kernel_hedgehog__glu_gated_swiglu__prompt_kernel(
        A_x, A_wqkv, A_w_phi, A_wo, B_x, B_w1, B_w3, B_w2):
    return build(A_x, A_wqkv, A_w_phi, A_wo, B_x, B_w1, B_w3, B_w2)
```

```python
import functools
import math
import jax
import jax.numpy as jnp
from jax import lax
import jax.experimental.pallas as pl
import jax.experimental.pallas.tpu as pltpu

S, D, H, DH, F = 2048, 640, 32, 20, 1536
NP = H // 2
PR = 2 * DH
NT_DIMS = (((1,), (1,)), ((), ()))
BF = jnp.bfloat16
F32 = jnp.float32
EPS = 1e-5
LOG2E = 1.4426950408889634


def _rcp(x):
    r = pl.reciprocal(x, approx=True)
    return r * (2.0 - x * r)


def _ln(x):
    m = jnp.mean(x, axis=-1, keepdims=True)
    xc = x - m
    v = jnp.mean(xc * xc, axis=-1, keepdims=True)
    return xc * lax.rsqrt(v + EPS)


def _red(x3, op):
    r = op(op(op(x3[0], x3[1]), op(x3[2], x3[3])), x3[4])
    r = op(r, pltpu.roll(r, 2, 0))
    r = op(r, pltpu.roll(r, 4, 0))
    return r


def _feat(p, T):
    p3 = p.reshape(5, 8, T)
    mx = _red(p3, jnp.maximum)
    mn = _red(p3, jnp.minimum)
    ep = jnp.exp2(p3 - mx[None])
    en = jnp.exp2(mn[None] - p3)
    rp = _rcp(_red(ep, jnp.add))
    rn = _rcp(_red(en, jnp.add))
    phi = jnp.concatenate([ep * rp[None], en * rn[None]], axis=0)
    return phi.reshape(2 * PR, T).astype(BF)


def _kernel(x_hbm, wqkv_hbm, wphi_hbm, wo_hbm, w1_hbm, w3_hbm, w2_hbm, out_hbm,
            x_v, out_v, xn_v, xz_v, vt_v, vz_v, wphi_v, wqkv_v, wo_v, w1_v, w3_v, w2_v, wt_v, wp_v, y_v, phiq_v, kv_acc, kvb_v,
            sems, *, TA, TB, SB, FC, XA, OSPLIT, N2, ORD, VW, L1, VT):
    NA = S // TA
    NB = S // TB

    def wcopy(c0, n, sem):
        return pltpu.make_async_copy(wqkv_hbm.at[:, pl.ds(c0, n)], wqkv_v.at[:, pl.ds(c0, n)], sems.at[sem])

    def xcopy(i):
        return pltpu.make_async_copy(x_hbm.at[pl.ds(i * TA, TA)], x_v.at[pl.ds(i * TA, TA)],
                                     sems.at[4 if i == 1 else 1])

    def ocopy(r, n):
        return pltpu.make_async_copy(out_v.at[pl.ds(r, n)], out_hbm.at[pl.ds(r, n)], sems.at[3])

    cp_qk = wcopy(0, 2 * D, 0)
    cp_va1 = wcopy(2 * D + 512, 128, 1)
    cp_va2 = wcopy(2 * D + 256, 256, 2)
    cp_vb = wcopy(2 * D, 256, 3)
    cp_xa = pltpu.make_async_copy(x_hbm.at[pl.ds(0, XA)], x_v.at[pl.ds(0, XA)], sems.at[0])
    cp_xb = pltpu.make_async_copy(x_hbm.at[pl.ds(XA, TA - XA)], x_v.at[pl.ds(XA, TA - XA)], sems.at[3])
    cp_phi = pltpu.make_async_copy(wphi_hbm, wphi_v, sems.at[0])
    cp_wo = pltpu.make_async_copy(wo_hbm, wo_v, sems.at[2])
    cp_w1 = pltpu.make_async_copy(w1_hbm, w1_v, sems.at[2])
    cp_w3 = pltpu.make_async_copy(w3_hbm, w3_v, sems.at[2])
    cp_w2 = pltpu.make_async_copy(w2_hbm, w2_v, sems.at[2])

    def proj(s, xn):
        return lax.dot_general(wt_v[pl.ds(D * s, D), :], xn, NT_DIMS, preferred_element_type=F32)

    def dot2(w, xn):
        tiles = (xn.shape[0] // 128) * (xn.shape[1] // 128)
        ns = 2 if tiles == 5 and w.shape[1] == 128 else 4 // math.gcd(4, tiles)
        m = w.shape[0] // ns
        return jnp.concatenate([lax.dot_general(w[m * u:m * (u + 1)], xn, NT_DIMS, preferred_element_type=F32)
                                for u in range(ns)], axis=0)

    def vstore(pv, p0, c0, n, vt_v=vt_v):
        ones = jnp.ones((8, n), F32)
        for p in range(pv.shape[0] // PR):
            vt_v[p0 + p, :, pl.ds(c0, n)] = jnp.concatenate([pv[PR * p:PR * (p + 1)], ones], axis=0).astype(BF)

    def vproj(xn):
        vstore(proj(2, xn), 0, 0, TA)

    def vrows(r0, n, xn):
        return lax.dot_general(wt_v[pl.ds(2 * D + r0, n), :], xn, NT_DIMS, preferred_element_type=F32)

    def transpose_v(c0, n):
        wt_v[pl.ds(2 * D + c0, n), :] = wqkv_v[:, pl.ds(2 * D + c0, n)].astype(F32).T.astype(BF)

    def fold(As, s):
        prev = None
        for t in range(5):
            w = wqkv_v[:, pl.ds(D * s + 128 * t, 128)]
            res = dot2(As[t], w)
            if prev is not None:
                res = jnp.concatenate([res[:PR] + prev, res[PR:]], axis=0)
            n = 160 if t == 4 else 120
            wt_v[pl.ds(D * s + 120 * t, n), :] = (res[:n] * LOG2E).astype(BF)
            prev = res[120:]

    def kstep(xn):
        pk = proj(1, xn)
        return [_feat(pk[PR * p:PR * (p + 1)], TA) for p in range(NP)]

    def qstep(xn, col):
        pq = proj(0, xn)
        for p in range(NP):
            phiq_v[pl.ds(2 * PR * p, 2 * PR), pl.ds(col, TA)] = _feat(pq[PR * p:PR * (p + 1)], TA)

    def astep(vts, phiks, first=False, last=False):
        if last:
            rr = lax.broadcasted_iota(jnp.int32, (48, 2 * PR), 0)
            cc = lax.broadcasted_iota(jnp.int32, (48, 2 * PR), 1)
            head_r = jnp.where(rr < PR, rr // DH, (rr - PR) // 4)
            mask = head_r == cc % 2
        for p in range(NP):
            kv = lax.dot_general(vts[p], phiks[p], NT_DIMS, preferred_element_type=F32)
            if not first:
                kv = kv + kv_acc[p]
            if last:
                kvb_v[p] = jnp.where(mask, kv, 0.0).astype(BF)
            else:
                kv_acc[p] = kv

    def vstep(row):
        xn1 = _ln(x_v[pl.ds(row, TA), :].astype(F32)).astype(BF)
        xn_v[...] = xn1
        vproj(xn1)

    def lnt(dst, r0, c, n=128):
        dst[pl.ds(128 * c, n), :] = _ln(x_v[pl.ds(r0 + 128 * c, n), :].astype(F32)).astype(BF)

    with jax.named_scope("prologue"):
        cp_xa.start(); cp_va1.start(); cp_va2.start(); cp_xb.start(); cp_vb.start(); xcopy(1).start()

        c8 = lax.broadcasted_iota(jnp.int32, (8, D), 1)
        r8 = lax.broadcasted_iota(jnp.int32, (8, D), 0)
        ch = c8 // DH
        cd = c8 - ch * DH
        key = ch + H * (cd % 4) - r8
        Y = jnp.concatenate([jnp.where(key == 8 * j, 1.0, 0.0) for j in range(16)], axis=0).astype(BF)
        cg = cd // 4
        hp = ch - r8 % 2
        y_v[...] = Y
        with jax.named_scope("w_xa"):
            cp_xa.wait()
        cp_phi.start(); cp_qk.start()
        lnt(xz_v, 0, 0, L1)
        with jax.named_scope("w_va1"):
            cp_va1.wait()
        for i in range(2, NA):
            xcopy(i).start()
        transpose_v(512, 128)
        if L1 < XA:
            lnt(xz_v, 0, L1 // 128, XA - L1)

        def vtop(c):
            xn = xz_v[pl.ds(128 * c, 128), :]
            pv = jnp.concatenate([vrows(512, 64, xn), vrows(576, 64, xn)], axis=0)
            vstore(pv[8:], 13, 128 * c, 128, vz_v)
            return pv[:8]

        tops = [vtop(c) for c in range(N2)]
        with jax.named_scope("w_va2"):
            cp_va2.wait()
        cp_wo.start(); cp_w1.start(); cp_w3.start(); cp_w2.start()
        tops += [vtop(c) for c in range(N2, 3)]
        xna = xz_v[pl.ds(0, XA), :]
        transpose_v(384, 128)
        transpose_v(256, 128)
        vstore(jnp.concatenate([vrows(400, 112, xna), jnp.concatenate(tops, axis=1)], axis=0), 10, 0, XA, vz_v)
        vstore(vrows(320, 80, xna), 8, 0, XA, vz_v)
        with jax.named_scope("w_b"):
            cp_xb.wait(); cp_vb.wait()
        xna = xz_v[pl.ds(0, XA), :]
        p3 = vrows(256, 64, xna)
        transpose_v(128, 128)
        transpose_v(0, 128)
        vstore(jnp.concatenate([vrows(160, 96, xna), p3], axis=0), 4, 0, XA, vz_v)
        vstore(vrows(80, 80, xna), 2, 0, XA, vz_v)
        vstore(vrows(0, 80, xna), 0, 0, XA, vz_v)
        lnt(xz_v, 0, 3)
        xnb = xz_v[pl.ds(XA, TA - XA), :]
        for g in range(8 - VW):
            vstore(vrows(80 * g, 80, xnb), 2 * g, XA, TA - XA, vz_v)
        with jax.named_scope("w_x1"):
            xcopy(1).wait()
        xnb = xz_v[pl.ds(XA, TA - XA), :]
        if VW == 8:
            for g in range(4):
                vstore(vrows(160 * g, 160, xnb), 4 * g, XA, TA - XA, vz_v)
        else:
            for g in range(8 - VW, 8):
                vstore(vrows(80 * g, 80, xnb), 2 * g, XA, TA - XA, vz_v)

        def vtile(c, g0=0, g1=4):
            xn = xn_v[pl.ds(VT * c, VT), :]
            for g in range(g0, g1):
                vstore(vrows(160 * g, 160, xn), 4 * g, VT * c, VT)

        for c in range(TA // VT):
            lnt(xn_v, TA, c * VT // 128, VT)
        cl = TA // VT - 1
        ga, gb = (0, 2) if VT == 128 else (2, 3)
        for c in range(cl):
            vtile(c)
        vtile(cl, 0, ga)
        with jax.named_scope("w_qk"):
            cp_phi.wait(); cp_qk.wait()
        vtile(cl, ga, gb)
        w = wphi_v[...].astype(F32)
        for g in range(5):
            vk = jnp.concatenate([w[4 * g + l] for l in range(4)], axis=1)
            wp_v[g, pl.ds(0, DH, stride=2), :] = vk
            wp_v[g, pl.ds(1, DH, stride=2), :] = vk
        C = jnp.dot(wp_v[...].reshape(5 * PR, 128).astype(BF), y_v[...], preferred_element_type=F32)
        vtile(cl, gb, 4)
        C = C.reshape(5, 5, 8, D)
        B2 = C[0]
        for g in range(1, 5):
            B2 = jnp.where((cg == g)[None], C[g], B2)
        As = []
        for t in range(5):
            b2 = B2[:, :, 128 * t:128 * (t + 1)]
            hpt = hp[:, 128 * t:128 * (t + 1)]
            a = jnp.concatenate([jnp.where((hpt == 2 * (3 * t + u))[None], b2, 0.0) for u in range(4)], axis=0)
            As.append(a.reshape(4 * PR, 128).astype(BF))
        for o in ORD:
            if o == "k":
                fold(As, 1)
            elif o == "q":
                fold(As, 0)
            elif o == "K":
                phiks0 = kstep(xz_v[...])
            elif o == "Q":
                qstep(xz_v[...], 0)
            else:
                astep([vz_v[p] for p in range(NP)], phiks0, first=True)

    def body_a(i, carry, last=False):
        if not last:
            @pl.when(i == 1)
            def _():
                for t in range(2, NA):
                    xcopy(t).wait()

            @pl.when(i == NA - 2)
            def _():
                cp_wo.wait(); cp_w1.wait(); cp_w3.wait(); cp_w2.wait()
        xn = xn_v[...]
        vts = [vt_v[p] for p in range(NP)]
        qstep(xn, i * TA if last else pl.multiple_of(i * TA, TA))
        phiks = kstep(xn)
        astep(vts, phiks, last=last)
        if not last:
            vstep(pl.multiple_of((i + 1) * TA, TA))
        return carry

    with jax.named_scope("phaseA"):
        lax.fori_loop(1, NA - 1, body_a, 0)
        body_a(NA - 1, 0, last=True)

    def attn(row):
        sub = lax.broadcasted_iota(jnp.int32, (8, SB), 0)
        ots = []
        for p in range(NP):
            nd = jnp.dot(kvb_v[p], phiq_v[pl.ds(2 * PR * p, 2 * PR), pl.ds(row, SB)],
                         preferred_element_type=F32)
            r = _rcp(nd[PR:PR + 8] + 1e-6)
            rs = pltpu.roll(r, 4, 0)
            ra = jnp.where(sub < 4, r, rs)
            rb = jnp.where(sub < 4, rs, r)
            ots.append(nd[:PR] * jnp.concatenate([ra, ra, r, rb, rb], axis=0))
        return jnp.concatenate(ots, axis=0).T.astype(BF)

    def oproj(row, o):
        h = x_v[pl.ds(row, SB), :].astype(F32) + jnp.dot(o, wo_v[...], preferred_element_type=F32)
        return h, _ln(h).astype(BF)

    def ffn(h, hn, row, splits):
        acc = h
        nc = F // FC
        for c in range(nc):
            gate = jnp.dot(hn, w1_v[:, pl.ds(FC * c, FC)], preferred_element_type=F32)
            up = jnp.dot(hn, w3_v[:, pl.ds(FC * c, FC)], preferred_element_type=F32)
            hg = 0.5 * gate
            act = ((hg + hg * jnp.tanh(hg)) * up).astype(BF)
            if c + 1 < nc:
                acc = acc + jnp.dot(act, w2_v[pl.ds(FC * c, FC), :], preferred_element_type=F32)
        r0 = 0
        for n in splits:
            res = acc[r0:r0 + n] + jnp.dot(act[r0:r0 + n], w2_v[pl.ds(F - FC, FC), :], preferred_element_type=F32)
            rw = pl.multiple_of(row + r0, 64)
            out_v[pl.ds(rw, n), :] = res.astype(BF)
            ocopy(rw, n).start()
            r0 += n

    nsub = TB // SB
    splits = [(SB,)] * (nsub - 1) + [OSPLIT]

    def body_b(j, carry):
        rows = [pl.multiple_of(j * TB + s * SB, SB) for s in range(nsub)]
        os_ = [attn(r) for r in rows]
        hs = [oproj(r, o) for r, o in zip(rows, os_)]
        for s in range(nsub):
            ffn(*hs[s], rows[s], splits[s])
        return carry

    with jax.named_scope("phaseB"):
        lax.fori_loop(0, NB, body_b, 0)

    with jax.named_scope("tail"):
        for j in range(NB):
            r0 = j * TB
            for sp in splits:
                for n in sp:
                    ocopy(r0, n).wait()
                    r0 += n


def build(A_x, A_wqkv, A_w_phi, A_wo, B_x, B_w1, B_w3, B_w2, TA=512, TB=512, SB=256, FC=512, XA=384, OS=2, N2=2, ORD='kqQKA', VW=6, L1=256, VT=128):
    OSPLIT = {0: (256,), 1: (128, 128), 2: (128, 64, 64), 3: (192, 64)}[OS]
    x2 = A_x.reshape(S, D)
    wphi_t = A_w_phi.transpose(1, 2, 0)
    any_spec = pl.BlockSpec(memory_space=pl.ANY)
    out = pl.pallas_call(
        functools.partial(_kernel, TA=TA, TB=TB, SB=SB, FC=FC, XA=XA, OSPLIT=OSPLIT, N2=N2, ORD=ORD, VW=VW, L1=L1, VT=VT),
        in_specs=[any_spec] * 7,
        out_specs=any_spec,
        out_shape=jax.ShapeDtypeStruct((S, D), BF),
        scratch_shapes=[
            pltpu.VMEM((S, D), BF),
            pltpu.VMEM((S, D), BF),
            pltpu.VMEM((TA, D), BF),
            pltpu.VMEM((TA, D), BF),
            pltpu.VMEM((NP, 48, TA), BF),
            pltpu.VMEM((NP, 48, TA), BF),
            pltpu.VMEM((DH, DH, H), BF),
            pltpu.VMEM((D, 3 * D), BF),
            pltpu.VMEM((D, D), BF),
            pltpu.VMEM((D, F), BF),
            pltpu.VMEM((D, F), BF),
            pltpu.VMEM((F, D), BF),
            pltpu.VMEM((3 * D, D), BF),
            pltpu.VMEM((5, PR, 128), F32),
            pltpu.VMEM((128, D), BF),
            pltpu.VMEM((2 * D, S), BF),
            pltpu.VMEM((NP, 48, 2 * PR), F32),
            pltpu.VMEM((NP, 48, 2 * PR), BF),
            pltpu.SemaphoreType.DMA((5,)),
        ],
        compiler_params=pltpu.CompilerParams(
            vmem_limit_bytes=100 * 1024 * 1024,
        ),
    )(x2, A_wqkv, wphi_t, A_wo, B_w1, B_w3, B_w2)
    return out.reshape(1, S, D)


@jax.jit
def pallas_sequential_preLN__linear_kernel_hedgehog__glu_gated_swiglu__prompt_kernel(
        A_x, A_wqkv, A_w_phi, A_wo, B_x, B_w1, B_w3, B_w2):
    return build(A_x, A_wqkv, A_w_phi, A_wo, B_x, B_w1, B_w3, B_w2)
```

```python
import functools
import math
import jax
import jax.numpy as jnp
from jax import lax
import jax.experimental.pallas as pl
import jax.experimental.pallas.tpu as pltpu

S, D, H, DH, F = 2048, 640, 32, 20, 1536
NP = H // 2
PR = 2 * DH
NS = 5
NG = 2 * NS + 1
NT_DIMS = (((1,), (1,)), ((), ()))
BF = jnp.bfloat16
F32 = jnp.float32
EPS = 1e-5
LOG2E = 1.4426950408889634


def _rcp(x):
    r = pl.reciprocal(x, approx=True)
    return r * (2.0 - x * r)


def _ln(x):
    m = jnp.mean(x, axis=-1, keepdims=True)
    xc = x - m
    v = jnp.mean(xc * xc, axis=-1, keepdims=True)
    return xc * lax.rsqrt(v + EPS)


def _red(x3, op):
    r = op(op(op(x3[0], x3[1]), op(x3[2], x3[3])), x3[4])
    r = op(r, pltpu.roll(r, 2, 0))
    r = op(r, pltpu.roll(r, 4, 0))
    return r


def _feat(p, T):
    p3 = p.reshape(5, 8, T)
    mx = _red(p3, jnp.maximum)
    mn = _red(p3, jnp.minimum)
    ep = jnp.exp2(p3 - mx[None])
    en = jnp.exp2(mn[None] - p3)
    rp = _rcp(_red(ep, jnp.add))
    rn = _rcp(_red(en, jnp.add))
    phi = jnp.concatenate([ep * rp[None], en * rn[None]], axis=0)
    return phi.reshape(2 * PR, T).astype(BF)


def _feat_split(p, T):
    even = lax.broadcasted_iota(jnp.int32, (8, T), 0) % 2 == 0

    def red(x3, op):
        m0, m1 = op(x3[0], x3[1]), op(x3[2], x3[3])
        r = op(op(jnp.where(even, m0, m1), pltpu.roll(jnp.where(even, m1, m0), 1, 0)), x3[4])
        r = op(r, pltpu.roll(r, 2, 0))
        return op(r, pltpu.roll(r, 4, 0))

    def spread(r):
        rs = pltpu.roll(r, 1, 0)
        r0, r1 = jnp.where(even, r, rs), jnp.where(even, rs, r)
        return jnp.stack([r0, r0, r1, r1, r], axis=0)

    p3 = p.reshape(5, 8, T)
    ep = jnp.exp2(p3 - spread(red(p3, jnp.maximum)))
    en = jnp.exp2(spread(red(p3, jnp.minimum)) - p3)
    ep = ep * spread(_rcp(red(ep, jnp.add)))
    en = en * spread(_rcp(red(en, jnp.add)))
    out = [jnp.concatenate([ep[i:j], en[i:j]], axis=0) for i, j in ((0, 2), (2, 4), (4, 5))]
    return [o.reshape(-1, T).astype(BF) for o in out]


def _kernel(x_hbm, wqkv_hbm, wphi_hbm, wo_hbm, w1_hbm, w3_hbm, w2_hbm, out_hbm,
            x_v, out_v, xn_v, vt_v, wphi_v, wqkv_v, wo_v, w1_v, w3_v, w2_v, wt_v, wp_v, wn_v, y_v, kvb_v, kvl_v, mk_v, va_v,
            sems, *, TA, TB, SB, FC, OSPLIT, ORB, WP, PRO):
    NB = S // TB

    def wcopy(c0, n, sem):
        return pltpu.make_async_copy(wqkv_hbm.at[:, pl.ds(c0, n)], wqkv_v.at[:, pl.ds(c0, n)], sems.at[sem])

    def xcopy(r0, r1, sem):
        return pltpu.make_async_copy(x_hbm.at[pl.ds(r0, r1 - r0)], x_v.at[pl.ds(r0, r1 - r0)], sems.at[sem])

    def ocopy(r, n, c0=0, nc=D):
        return pltpu.make_async_copy(out_v.at[pl.ds(r, n), pl.ds(c0, nc)], out_hbm.at[pl.ds(r, n), pl.ds(c0, nc)],
                                     sems.at[1])

    def vcopy(r0, n, sem):
        return pltpu.make_async_copy(wqkv_hbm.at[pl.ds(r0, n), pl.ds(2 * D, D)],
                                     wqkv_v.at[pl.ds(r0, n), pl.ds(2 * D, D)], sems.at[sem])

    groups, nx, nk = [], 0, 0
    for g, (pieces, _, _) in enumerate(PRO):
        cps, sem = [], g % (len(PRO) - 1)
        for kind, n in pieces:
            if kind == "x":
                cps.append(xcopy(128 * nx, 128 * (nx + n), sem))
                nx += n
            elif kind == "k":
                cps.append(vcopy(128 * nk, 128 * n, sem))
                nk += n
            elif kind == "p":
                cps.append(pltpu.make_async_copy(wphi_hbm, wphi_v, sems.at[sem]))
            else:
                cps.append(wcopy(0, 2 * D, sem))
        groups.append(cps)
    assert nk == 5 and 128 * nx == S
    cp_wo = pltpu.make_async_copy(wo_hbm, wo_v, sems.at[1])
    cp_w1 = pltpu.make_async_copy(w1_hbm, w1_v, sems.at[1])
    cp_w3 = pltpu.make_async_copy(w3_hbm, w3_v, sems.at[1])
    cp_w2 = pltpu.make_async_copy(w2_hbm, w2_v, sems.at[1])

    def wstart():
        cp_wo.start(); cp_w1.start(); cp_w3.start(); cp_w2.start()

    def dot2(w, xn):
        tiles = (xn.shape[0] // 128) * (xn.shape[1] // 128)
        ns = 2 if tiles == 5 and w.shape[1] == 128 else 4 // math.gcd(4, tiles)
        m = w.shape[0] // ns
        return jnp.concatenate([lax.dot_general(w[m * u:m * (u + 1)], xn, NT_DIMS, preferred_element_type=F32)
                                for u in range(ns)], axis=0)

    def vstore(pv, c0, n):
        low = lax.broadcasted_iota(jnp.int32, (8, n), 0) < 4
        for q in range(NS):
            r = 120 * q
            mid = pv[r + 56:r + 64]
            vt_v[2 * q, :, pl.ds(c0, n)] = jnp.concatenate(
                [pv[r:r + 56], jnp.where(low, mid, 1.0)], axis=0).astype(BF)
            vt_v[2 * q + 1, :, pl.ds(c0, n)] = jnp.concatenate(
                [jnp.where(low, 1.0, mid), pv[r + 64:r + 120]], axis=0).astype(BF)
        vt_v[NG - 1, pl.ds(0, 48), pl.ds(c0, n)] = jnp.concatenate(
            [pv[D - PR:], jnp.ones((8, n), F32)], axis=0).astype(BF)

    def vrows(r0, n, xn):
        return lax.dot_general(wt_v[pl.ds(2 * D + r0, n), :], xn, NT_DIMS, preferred_element_type=F32)

    def transpose_v(k):
        wt_v[pl.ds(2 * D, D), pl.ds(128 * k, 128)] = (
            wqkv_v[pl.ds(128 * k, 128), pl.ds(2 * D, D)].astype(F32).T.astype(BF))

    def vdot(c, nt, k, nk):
        return dot2(wt_v[pl.ds(2 * D, D), pl.ds(128 * k, 128 * nk)],
                    xn_v[pl.ds(128 * c, 128 * nt), pl.ds(128 * k, 128 * nk)])

    def fold(As, s):
        prev = None
        for t in range(5):
            w = wqkv_v[:, pl.ds(D * s + 128 * t, 128)]
            res = dot2(As[t], w)
            if prev is not None:
                res = jnp.concatenate([res[:PR] + prev, res[PR:]], axis=0)
            n = 160 if t == 4 else 120
            wt_v[pl.ds(D * s + 120 * t, n), :] = (res[:n] * LOG2E).astype(BF)
            prev = res[120:]

    def feats(s, row, n):
        pk = dot2(wt_v[pl.ds(D * s, D), :], xn_v[pl.ds(row, n), :])
        out = []
        for q in range(NS):
            r = 120 * q
            fa = _feat(pk[r:r + PR], n)
            f0, f1, fm = _feat_split(pk[r + PR:r + 2 * PR], n)
            fc = _feat(pk[r + 2 * PR:r + 3 * PR], n)
            out += [jnp.concatenate([fa, f0, fm], axis=0), jnp.concatenate([fc, f1, fm], axis=0)]
        return out + [_feat(pk[D - PR:], n)]

    def astep(kvs, b, phiks):
        out = []
        for g in range(NG):
            m = 64 if g < NG - 1 else 48
            kv = lax.dot_general(vt_v[g, pl.ds(0, m), pl.ds(TA * b, TA)], phiks[g], NT_DIMS,
                                 preferred_element_type=F32)
            out.append(kv if kvs is None else kv + kvs[g])
        return out

    def lnt(c, n=128):
        xn_v[pl.ds(128 * c, n), :] = _ln(x_v[pl.ds(128 * c, n), :].astype(F32)).astype(BF)

    with jax.named_scope("prologue"):
        for cps in groups[:-1]:
            for cp in cps:
                cp.start()

        c8 = lax.broadcasted_iota(jnp.int32, (8, D), 1)
        r8 = lax.broadcasted_iota(jnp.int32, (8, D), 0)
        ch = c8 // DH
        cd = c8 - ch * DH
        key = ch + H * (cd % 4) - r8
        Y = jnp.concatenate([jnp.where(key == 8 * j, 1.0, 0.0) for j in range(16)], axis=0).astype(BF)
        cg = cd // 4
        hp = ch - r8 % 2
        y_v[...] = Y
        wn_v[...] = jnp.zeros(wn_v.shape, F32)

        rr = lax.broadcasted_iota(jnp.int32, (64, 128), 0)
        cc = lax.broadcasted_iota(jnp.int32, (64, 128), 1)
        par = cc % 2
        for e in range(2):
            head_c = jnp.where(cc < 2 * PR, par, jnp.where((cc < 112) | (par == e), 2, 3))
            if e == 0:
                head_r = jnp.where(rr < 60, rr // DH, jnp.minimum(rr - 60, 2))
            else:
                head_r = (jnp.where(rr < 4, jnp.minimum(rr, 2), (rr - 4) // DH) + 2) % 3
            mk_v[e] = head_r - head_c
        mk_v[2] = jnp.where(rr < PR, rr // DH, (rr - PR) // 4) - par

        def cmat():
            w = wphi_v[...].astype(F32)
            for g in range(5):
                wn_v[g, pl.ds(0, DH), :] = jnp.concatenate([w[4 * g + l] for l in range(4)], axis=1)
            wn = wn_v[...].reshape(5 * 24, 128).astype(BF)
            c4 = [jnp.dot(wn[32 * u:min(32 * (u + 1), 120)], y_v[:, pl.ds(512, 128)], preferred_element_type=F32)
                  for u in range(4)]
            return jnp.concatenate([jnp.dot(wn, y_v[:, pl.ds(0, 512)], preferred_element_type=F32),
                                    jnp.concatenate(c4, axis=0)], axis=1)

        def abuild(C):
            C = C.reshape(5, 3, 8, D)
            B1 = C[0]
            for g in range(1, 5):
                B1 = jnp.where((cg == g)[None], C[g], B1)
            As = []
            for t in range(5):
                b1 = B1[:, :, 128 * t:128 * (t + 1)]
                b20 = b1.reshape(24, 128)[:DH]
                wp_v[t, pl.ds(0, DH, stride=2), :] = b20
                wp_v[t, pl.ds(1, DH, stride=2), :] = b20
                b2 = wp_v[t].reshape(5, 8, 128)
                hpt = hp[:, 128 * t:128 * (t + 1)]
                cht = ch[:, 128 * t:128 * (t + 1)]
                rows = []
                for u in range(4):
                    h0 = 2 * (3 * t + u)
                    if u == 1:
                        rows += [jnp.where((cht == h0)[None], b1[:2], 0.0),
                                 jnp.where((cht == h0 + 1)[None], b1[:2], 0.0),
                                 jnp.where((hpt == h0)[None], b2[4:], 0.0)]
                    else:
                        rows.append(jnp.where((hpt == h0)[None], b2, 0.0))
                As.append(jnp.concatenate(rows, axis=0).reshape(4 * PR, 128).astype(BF))
            return As

        done = [0] * (S // 128)
        nl = nt_ = nk = na = 0
        kvs, phiks, As = None, {}, None
        for g, (pieces, lns, units) in enumerate(PRO):
            with jax.named_scope(f"w_{g}"):
                for cp in groups[g]:
                    cp.wait()
            if g == 0:
                for cp in groups[-1]:
                    cp.start()
            if g == len(PRO) - 1:
                wstart()
            acc = {}
            news = sum(n for kind, n in pieces if kind == "k")
            for u in units:
                if u == "T":
                    for k in range(nt_, nt_ + news):
                        transpose_v(k)
                    nt_ += news
                    for c in range(nl, nl + lns):
                        lnt(c)
                    nl += lns
                elif u == "C":
                    C = cmat()
                elif u in ("k", "q"):
                    As = As or abuild(C)
                    fold(As, 1 if u == "k" else 0)
                elif u == "K":
                    phiks[nk] = feats(1, TA * nk, TA)
                    nk += 1
                elif u == "A":
                    assert all(d == 5 for d in done[4 * na:4 * na + 4])
                    kvs = astep(kvs, na, phiks.pop(na))
                    na += 1
                else:
                    c0, nt, k, n = u if len(u) == 4 else (u[0], 1, 0, 5)
                    for c in range(nl, c0 + nt):
                        lnt(c)
                    nl = max(nl, c0 + nt)
                    if n == 0:
                        continue
                    r = vdot(c0, nt, k, n)
                    for c in range(c0, c0 + nt):
                        rc = r[:, 128 * (c - c0):128 * (c - c0 + 1)]
                        if done[c]:
                            rc = rc + (acc[c] if c in acc else va_v[:, pl.ds(128 * (c % 5), 128)])
                        done[c] += n
                        acc[c] = rc
                        if done[c] == 5:
                            vstore(acc.pop(c), 128 * c, 128)
            for c, rc in acc.items():
                va_v[:, pl.ds(128 * (c % 5), 128)] = rc
        assert nl == S // 128 and nk == na == S // TA
        for g in range(NG - 1):
            kvb_v[g] = jnp.where(mk_v[g % 2] == 0, kvs[g], 0.0).astype(BF)
        kvl_v[...] = jnp.where(mk_v[2, pl.ds(0, 48), pl.ds(0, 2 * PR)] == 0, kvs[NG - 1], 0.0).astype(BF)
        with jax.named_scope("w_w"):
            cp_wo.wait(); cp_w1.wait(); cp_w3.wait(); cp_w2.wait()

    def attn(phiq):
        low = lax.broadcasted_iota(jnp.int32, (8, SB), 0) < 4
        ots = []
        for q in range(NS):
            n1 = jnp.dot(kvb_v[2 * q], phiq[2 * q], preferred_element_type=F32)
            n2 = jnp.dot(kvb_v[2 * q + 1], phiq[2 * q + 1], preferred_element_type=F32)
            r = _rcp(jnp.where(low, n2[:8], n1[56:]) + 1e-6)
            ra, rb, rc, rd, re, rf = [jnp.broadcast_to(r[k:k + 1], (8, SB)) for k in (4, 5, 6, 0, 1, 2)]
            num = jnp.concatenate([n1[:56], jnp.where(low, n1[56:], n2[:8]), n2[8:]], axis=0)
            scale = jnp.concatenate([ra, ra, jnp.where(low, ra, rb), rb, rb, rc, rc, jnp.where(low, rc, rd),
                                     rd, rd, re, re, jnp.where(low, re, rf), rf, rf], axis=0)
            ots.append(num * scale)
        nd = jnp.dot(kvl_v[...], phiq[NG - 1], preferred_element_type=F32)
        r = _rcp(nd[PR:PR + 8] + 1e-6)
        rs = pltpu.roll(r, 4, 0)
        ra = jnp.where(low, r, rs)
        rb = jnp.where(low, rs, r)
        ots.append(nd[:PR] * jnp.concatenate([ra, ra, r, rb, rb], axis=0))
        return jnp.concatenate(ots, axis=0).T.astype(BF)

    def oproj(row, o):
        hs, hns = [], []
        m = SB // WP
        for u in range(WP):
            rw = pl.multiple_of(row + m * u, m)
            h = x_v[pl.ds(rw, m), :].astype(F32) + jnp.dot(o[m * u:m * (u + 1)], wo_v[...], preferred_element_type=F32)
            hs.append(h)
            hns.append(_ln(h).astype(BF))
        return jnp.concatenate(hs, axis=0), jnp.concatenate(hns, axis=0)

    def ffn(h, hn, row, splits):
        acc = h
        nc = F // FC
        for c in range(nc):
            gate = jnp.dot(hn, w1_v[:, pl.ds(FC * c, FC)], preferred_element_type=F32)
            up = jnp.dot(hn, w3_v[:, pl.ds(FC * c, FC)], preferred_element_type=F32)
            hg = 0.5 * gate
            act = ((hg + hg * jnp.tanh(hg)) * up).astype(BF)
            if c + 1 < nc:
                acc = acc + jnp.dot(act, w2_v[pl.ds(FC * c, FC), :], preferred_element_type=F32)
        r0 = 0
        for n, cols in splits:
            rw = pl.multiple_of(row + r0, 64)
            c0 = 0
            for nc in cols:
                res = acc[r0:r0 + n, c0:c0 + nc] + jnp.dot(act[r0:r0 + n], w2_v[pl.ds(F - FC, FC), pl.ds(c0, nc)],
                                                           preferred_element_type=F32)
                out_v[pl.ds(rw, n), pl.ds(c0, nc)] = res.astype(BF)
                ocopy(rw, n, c0, nc).start()
                c0 += nc
            r0 += n

    nsub = TB // SB
    splits = [((SB, (D,)),)] * (nsub - 1) + [OSPLIT]

    def body_b(j, carry):
        rows = [pl.multiple_of(j * TB + s * SB, SB) for s in range(nsub)]
        qs, os_, hs, nf = [], [], [], 0
        for o in ORB:
            if o == "Q":
                qs.append(feats(0, rows[len(qs)], SB))
            elif o == "A":
                os_.append(attn(qs[len(os_)]))
            elif o == "W":
                hs.append(oproj(rows[len(hs)], os_[len(hs)]))
            else:
                ffn(*hs[nf], rows[nf], splits[nf])
                nf += 1
        assert nf == nsub
        return carry

    with jax.named_scope("phaseB"):
        lax.fori_loop(0, NB, body_b, 0)

    with jax.named_scope("tail"):
        for j in range(NB):
            r0 = j * TB
            for sp in splits:
                for n, cols in sp:
                    c0 = 0
                    for nc in cols:
                        ocopy(r0, n, c0, nc).wait()
                        c0 += nc
                    r0 += n


def _full(c0, c1):
    return [(c,) for c in range(c0, c1)]


_HEAD = {
    0: [([("x", 3)], 2, ["T"]),
        ([("k", 1)], 1, ["T", (0, 2, 0, 1)]),
        ([("x", 1), ("k", 2)], 1, [(2, 1, 0, 1), "T", (0, 3, 1, 2), (3, 1, 0, 2)]),
        ([("x", 1), ("k", 2)], 1, [(3, 1, 2, 1), "T", (0, 4, 3, 2)]),
        ([("x", 6)], 0, [(4,)])],
    7: [([("x", 3)], 2, ["T"]),
        ([("k", 1)], 1, ["T", (0, 2, 0, 1)]),
        ([("k", 1), ("x", 2)], 2, [(2, 1, 0, 1), "T", (0, 3, 1, 1), (3, 1, 0, 2)]),
        ([("k", 3)], 0, [(4, 1, 0, 2), "T", (0, 5, 2, 2), (0, 1, 4, 1)]),
        ([("x", 6)], 0, [(1, 4, 4, 1)])],
    8: [([("x", 3)], 2, ["T"]),
        ([("k", 1)], 1, ["T", (0, 2, 0, 1)]),
        ([("k", 1), ("x", 2)], 2, [(2, 1, 0, 1), "T", (0, 3, 1, 1), (3, 1, 0, 2)]),
        ([("k", 3)], 0, [(4, 1, 0, 2), "T", (0, 4, 2, 3)]),
        ([("x", 6)], 0, [(4, 1, 2, 3)])],
}
_HEAD[2] = [([("x", 3)], 2, ["T"]),
            ([("k", 1)], 1, ["T", (0, 2, 0, 1)]),
            ([("k", 1), ("x", 1)], 1, [(2, 1, 0, 1), "T", (0, 3, 1, 1), (3, 1, 0, 1)]),
            ([("k", 3), ("x", 1)], 1, [(3, 1, 1, 1), "T", (0, 4, 2, 3)]),
            ([("x", 6)], 0, [(4,)])]
_HEAD[11] = [([("x", 3)], 2, ["T"]),
             ([("k", 1)], 1, ["T", (0, 2, 0, 1)]),
             ([("k", 1), ("x", 2)], 2, [(2, 1, 0, 1), "T", (0, 3, 1, 1), (3, 1, 0, 2)]),
             ([("k", 3)], 0, [(4, 1, 0, 1), "T", (0, 4, 2, 3)]),
             ([("x", 6)], 0, [(4, 1, 1, 4)])]
_HEAD[12] = [([("x", 3)], 2, ["T"]),
             ([("k", 1)], 1, ["T", (0, 2, 0, 1)]),
             ([("k", 1), ("x", 2)], 2, [(2, 1, 0, 1), "T", (0, 3, 1, 1), (3, 1, 0, 1)]),
             ([("k", 3)], 0, [(3, 1, 1, 1), "T", (0, 4, 2, 3)]),
             ([("x", 6)], 0, [(4,)])]
_HEAD[13] = [([("x", 3)], 2, ["T"]),
             ([("k", 1)], 1, ["T", (0, 2, 0, 1)]),
             ([("k", 1), ("x", 1)], 1, [(2, 1, 0, 1), "T", (0, 3, 1, 1), (3, 1, 0, 2)]),
             ([("k", 2), ("x", 1), ("k", 1)], 1, ["T", (0, 4, 2, 1), (0, 4, 3, 2)]),
             ([("x", 6)], 0, [(4,)])]
_MID = {
    0: ([(9,), (10, 1, 0, 0)], [(10, 1, 0, 2), "C", (10, 1, 2, 3)]),
    1: ([(9, 1, 0, 3), (10, 1, 0, 2)], [(9, 1, 3, 2), "C", (10, 1, 2, 3)]),
    2: ([(9, 2, 0, 3)], [(9, 1, 3, 2), "C", (10, 1, 3, 2)]),
    3: ([(9,), (10, 1, 0, 1)], [(10, 1, 1, 2), "C", (10, 1, 3, 2)]),
    4: ([(9, 2, 0, 2)], [(9, 1, 2, 3), "C", (10, 1, 2, 3)]),
}


def _tokens(order, c):
    out = []
    for o in order:
        if o.isdigit():
            out.append((c, int(o), 0, 5))
            c += int(o)
        else:
            out.append(o)
    return out


def build(A_x, A_wqkv, A_w_phi, A_wo, B_x, B_w1, B_w3, B_w2, TA=512, TB=512, SB=256, FC=512, OS=5,
          ORD='k1q1111KKAAKKAA', ORB='QQAAWWFF', WP=4, NBC=0, PR_=0, MID=1):
    PRO = [list(e) for e in _HEAD[PR_]]
    PRO[-1][2] = PRO[-1][2] + _full(5, 9) + _MID[MID][0]
    PRO.append([[("p", 0), ("w", 0), ("x", 5)], 0, _MID[MID][1] + _tokens(ORD, 11)])
    OSPLIT = {2: ((128, (D,)), (64, (D,)), (64, (D,))),
              4: ((128, (D,)), (64, (D,)), (64, (512, 128))),
              5: ((128, (D,)), (64, (D,)), (64, (384, 128, 128))),
              6: ((128, (D,)), (128, (384, 128, 128))),
              7: ((128, (D,)), (128, (256, 128, 128, 128))),
              8: ((192, (D,)), (64, (384, 128, 128))),
              9: ((256, (256, 128, 128, 128)),),
              10: ((128, (D,)), (64, (D,)), (64, (384, 256))),
              }[OS]
    x2 = A_x.reshape(S, D)
    wphi_t = A_w_phi.transpose(1, 2, 0)
    any_spec = pl.BlockSpec(memory_space=pl.ANY)
    out = pl.pallas_call(
        functools.partial(_kernel, TA=TA, TB=TB, SB=SB, FC=FC, OSPLIT=OSPLIT, ORB=ORB, WP=WP, PRO=PRO),
        in_specs=[any_spec] * 7,
        out_specs=any_spec,
        out_shape=jax.ShapeDtypeStruct((S, D), BF),
        scratch_shapes=[
            pltpu.VMEM((S, D), BF),
            pltpu.VMEM((S, D), BF),
            pltpu.VMEM((S, D), BF),
            pltpu.VMEM((NG, 64, S), BF),
            pltpu.VMEM((DH, DH, H), BF),
            pltpu.VMEM((D, 3 * D), BF),
            pltpu.VMEM((D, D), BF),
            pltpu.VMEM((D, F), BF),
            pltpu.VMEM((D, F), BF),
            pltpu.VMEM((F, D), BF),
            pltpu.VMEM((3 * D, D), BF),
            pltpu.VMEM((5, PR, 128), F32),
            pltpu.VMEM((5, 24, 128), F32),
            pltpu.VMEM((128, D), BF),
            pltpu.VMEM((NG - 1, 64, 128), BF),
            pltpu.VMEM((48, 2 * PR), BF),
            pltpu.VMEM((3, 64, 128), jnp.int32),
            pltpu.VMEM((D, 640), F32),
            pltpu.SemaphoreType.DMA((len(PRO) - 1,)),
        ],
        compiler_params=pltpu.CompilerParams(
            vmem_limit_bytes=100 * 1024 * 1024,
            disable_bounds_checks=bool(NBC),
        ),
    )(x2, A_wqkv, wphi_t, A_wo, B_w1, B_w3, B_w2)
    return out.reshape(1, S, D)


@jax.jit
def pallas_sequential_preLN__linear_kernel_hedgehog__glu_gated_swiglu__prompt_kernel(
        A_x, A_wqkv, A_w_phi, A_wo, B_x, B_w1, B_w3, B_w2):
    return build(A_x, A_wqkv, A_w_phi, A_wo, B_x, B_w1, B_w3, B_w2)
```

```python
import functools
import math
import jax
import jax.numpy as jnp
from jax import lax
import jax.experimental.pallas as pl
import jax.experimental.pallas.tpu as pltpu

S, D, H, DH, F = 2048, 640, 32, 20, 1536
PR = 2 * DH
NS = 5
NG = 2 * NS + 1
SEXT = ((2, 3, 4), (5, 6, 7), (8, 9, 10), (11, 12, 13), (0, 1, 14))
MIDS = tuple(m for _, m, _ in SEXT)
NT_DIMS = (((1,), (1,)), ((), ()))
BF = jnp.bfloat16
F32 = jnp.float32
EPS = 1e-5
LOG2E = 1.4426950408889634


def _rcp(x):
    r = pl.reciprocal(x, approx=True)
    return r * (2.0 - x * r)


def _ln(x):
    m = jnp.mean(x, axis=-1, keepdims=True)
    xc = x - m
    v = jnp.mean(xc * xc, axis=-1, keepdims=True)
    return xc * lax.rsqrt(v + EPS)


def _red(x3, op):
    r = op(op(op(x3[0], x3[1]), op(x3[2], x3[3])), x3[4])
    r = op(r, pltpu.roll(r, 2, 0))
    r = op(r, pltpu.roll(r, 4, 0))
    return r


def _feat(p, T):
    p3 = p.reshape(5, 8, T)
    mx = _red(p3, jnp.maximum)
    mn = _red(p3, jnp.minimum)
    ep = jnp.exp2(p3 - mx[None])
    en = jnp.exp2(mn[None] - p3)
    rp = _rcp(_red(ep, jnp.add))
    rn = _rcp(_red(en, jnp.add))
    phi = jnp.concatenate([ep * rp[None], en * rn[None]], axis=0)
    return phi.reshape(2 * PR, T)


def _feat_split(p, T):
    even = lax.broadcasted_iota(jnp.int32, (8, T), 0) % 2 == 0

    def red(x3, op):
        m0, m1 = op(x3[0], x3[1]), op(x3[2], x3[3])
        r = op(op(jnp.where(even, m0, m1), pltpu.roll(jnp.where(even, m1, m0), 1, 0)), x3[4])
        r = op(r, pltpu.roll(r, 2, 0))
        return op(r, pltpu.roll(r, 4, 0))

    def spread(r):
        rs = pltpu.roll(r, 1, 0)
        r0, r1 = jnp.where(even, r, rs), jnp.where(even, rs, r)
        return jnp.stack([r0, r0, r1, r1, r], axis=0)

    p3 = p.reshape(5, 8, T)
    ep = jnp.exp2(p3 - spread(red(p3, jnp.maximum)))
    en = jnp.exp2(spread(red(p3, jnp.minimum)) - p3)
    ep = ep * spread(_rcp(red(ep, jnp.add)))
    en = en * spread(_rcp(red(en, jnp.add)))
    out = [jnp.concatenate([ep[i:j], en[i:j]], axis=0) for i, j in ((0, 2), (2, 4), (4, 5))]
    return [o.reshape(-1, T) for o in out]


def _kernel(x_hbm, wqkv_hbm, wphi_hbm, wo_hbm, w1_hbm, w3_hbm, w2_hbm, out_hbm,
            x_v, out_v, xn_v, vt_v, wphi_v, wqkv_v, wo_v, w1_v, w3_v, w2_v, wt_v, wp_v, wn_v, y_v, kvb_v, kvl_v, mk_v, va_v, vn_v,
            sems, *, TA, TB, SB, FC, OSPLIT, ORB, WP, PRO):
    NB = S // TB

    def wcopy(c0, n, sem):
        return pltpu.make_async_copy(wqkv_hbm.at[:, pl.ds(c0, n)], wqkv_v.at[:, pl.ds(c0, n)], sems.at[sem])

    def xcopy(r0, r1, sem):
        return pltpu.make_async_copy(x_hbm.at[pl.ds(r0, r1 - r0)], x_v.at[pl.ds(r0, r1 - r0)], sems.at[sem])

    def ocopy(r, n, c0=0, nc=D):
        return pltpu.make_async_copy(out_v.at[pl.ds(r, n), pl.ds(c0, nc)], out_hbm.at[pl.ds(r, n), pl.ds(c0, nc)],
                                     sems.at[1])

    def vcopy(r0, n, sem):
        return pltpu.make_async_copy(wqkv_hbm.at[pl.ds(r0, n), pl.ds(2 * D, D)],
                                     wqkv_v.at[pl.ds(r0, n), pl.ds(2 * D, D)], sems.at[sem])

    groups, nx, nk = [], 0, 0
    for g, (pieces, _, _) in enumerate(PRO):
        cps, sem = [], g % (len(PRO) - 1)
        for kind, n in pieces:
            if kind == "x":
                cps.append(xcopy(128 * nx, 128 * (nx + n), sem))
                nx += n
            elif kind == "k":
                cps.append(vcopy(128 * nk, 128 * n, sem))
                nk += n
            elif kind == "p":
                cps.append(pltpu.make_async_copy(wphi_hbm, wphi_v, sems.at[sem]))
            else:
                cps.append(wcopy(0, 2 * D, sem))
        groups.append(cps)
    assert nk == 5 and 128 * nx == S
    cp_wo = pltpu.make_async_copy(wo_hbm, wo_v, sems.at[1])
    cp_w1 = pltpu.make_async_copy(w1_hbm, w1_v, sems.at[1])
    cp_w3 = pltpu.make_async_copy(w3_hbm, w3_v, sems.at[1])
    cp_w2 = pltpu.make_async_copy(w2_hbm, w2_v, sems.at[1])

    def wstart():
        cp_wo.start(); cp_w1.start(); cp_w3.start(); cp_w2.start()

    def dot2(w, xn, ms=None):
        tiles = (xn.shape[0] // 128) * (xn.shape[1] // 128)
        ns = 4 // math.gcd(4, tiles)
        ms = ms or [w.shape[0] // ns] * ns
        return jnp.concatenate([lax.dot_general(w[sum(ms[:u]):sum(ms[:u + 1])], xn, NT_DIMS,
                                                preferred_element_type=F32) for u in range(len(ms))], axis=0)

    def vstore(pv, c0, n):
        low = lax.broadcasted_iota(jnp.int32, (8, n), 0) < 4
        for q, (a, m, c) in enumerate(SEXT):
            r = PR * m
            mid = pv[r + 16:r + 24]
            vt_v[2 * q, :, pl.ds(c0, n)] = jnp.concatenate(
                [pv[PR * a:PR * (a + 1)], pv[r:r + 16], jnp.where(low, mid, 1.0)], axis=0).astype(BF)
            vt_v[2 * q + 1, :, pl.ds(c0, n)] = jnp.concatenate(
                [jnp.where(low, 1.0, mid), pv[r + 24:r + PR], pv[PR * c:PR * (c + 1)]], axis=0).astype(BF)
        vt_v[NG - 1, pl.ds(0, 48), pl.ds(c0, n)] = jnp.concatenate(
            [pv[D - PR:], jnp.ones((8, n), F32)], axis=0).astype(BF)

    def transpose_v(k):
        wt_v[pl.ds(2 * D, D), pl.ds(128 * k, 128)] = (
            wqkv_v[pl.ds(128 * k, 128), pl.ds(2 * D, D)].astype(F32).T.astype(BF))

    def vdot(c, nt, k, nk):
        return dot2(wt_v[pl.ds(2 * D, D), pl.ds(128 * k, 128 * nk)],
                    xn_v[pl.ds(128 * c, 128 * nt), pl.ds(128 * k, 128 * nk)])

    def ndot(c, nt, k, nk, ns):
        m = 128 * nt // ns
        return jnp.concatenate([jnp.dot(xn_v[pl.ds(128 * c + m * u, m), pl.ds(128 * k, 128 * nk)],
                                        wqkv_v[pl.ds(128 * k, 128 * nk), pl.ds(2 * D, D)],
                                        preferred_element_type=F32) for u in range(ns)], axis=0)

    def fold(As, s):
        prev = None
        for t in range(5):
            w = wqkv_v[:, pl.ds(D * s + 128 * t, 128)]
            res = dot2(As[t], w, [80, 80] if (s, t) == (1, 2) else [As[t].shape[0]])
            if t in (1, 2):
                res = jnp.concatenate([res[:16] + prev[:16], res[16:32], res[32:PR] + prev[16:], res[PR:]], axis=0)
            elif t > 2:
                res = jnp.concatenate([prev[:16], prev[16:] + res[:24], res[24:]], axis=0)
            n = 160 if t == 4 else 120
            wt_v[pl.ds(D * s + 120 * t, n), :] = (res[:n] * LOG2E).astype(BF)
            prev = res[120:]

    def feats(s, row, n):
        pk = dot2(wt_v[pl.ds(D * s, D), :], xn_v[pl.ds(row, n), :])
        out = []
        for a, m, c in SEXT:
            fa = _feat(pk[PR * a:PR * (a + 1)], n)
            f0, f1, fm = _feat_split(pk[PR * m:PR * (m + 1)], n)
            fc = _feat(pk[PR * c:PR * (c + 1)], n)
            out += [jnp.concatenate([fa, f0, fm], axis=0).astype(BF), jnp.concatenate([fc, f1, fm], axis=0).astype(BF)]
        return out + [_feat(pk[D - PR:], n).astype(BF)]

    def astep(kvs, b, phiks):
        out = []
        for g in range(NG):
            m = 64 if g < NG - 1 else 48
            kv = lax.dot_general(vt_v[g, pl.ds(0, m), pl.ds(TA * b, TA)], phiks[g], NT_DIMS,
                                 preferred_element_type=F32)
            out.append(kv if kvs is None else kv + kvs[g])
        return out

    def lnt(c, n=128):
        xn_v[pl.ds(128 * c, n), :] = _ln(x_v[pl.ds(128 * c, n), :].astype(F32)).astype(BF)

    with jax.named_scope("prologue"):
        for cps in groups[:-1]:
            for cp in cps:
                cp.start()

        c8 = lax.broadcasted_iota(jnp.int32, (8, D), 1)
        r8 = lax.broadcasted_iota(jnp.int32, (8, D), 0)
        ch = c8 // DH
        cd = c8 - ch * DH
        key = ch + H * (cd % 4) - r8
        Y = jnp.concatenate([jnp.where(key == 8 * j, 1.0, 0.0) for j in range(16)], axis=0).astype(BF)
        cg = cd // 4
        hp = ch - r8 % 2
        y_v[...] = Y
        wn_v[...] = jnp.zeros(wn_v.shape, F32)

        rr = lax.broadcasted_iota(jnp.int32, (64, 128), 0)
        cc = lax.broadcasted_iota(jnp.int32, (64, 128), 1)
        par = cc % 2
        for e in range(2):
            head_c = jnp.where(cc < 2 * PR, par, jnp.where((cc < 112) | (par == e), 2, 3))
            if e == 0:
                head_r = jnp.where(rr < 60, rr // DH, jnp.minimum(rr - 60, 2))
            else:
                head_r = (jnp.where(rr < 4, jnp.minimum(rr, 2), (rr - 4) // DH) + 2) % 3
            mk_v[e] = head_r - head_c
        mk_v[2] = jnp.where(rr < PR, rr // DH, (rr - PR) // 4) - par

        def cmat():
            w = wphi_v[...].astype(F32)
            for g in range(5):
                wn_v[g, pl.ds(0, DH), :] = jnp.concatenate([w[4 * g + l] for l in range(4)], axis=1)
            wn = wn_v[...].reshape(5 * 24, 128).astype(BF)
            c4 = [jnp.dot(wn[32 * u:min(32 * (u + 1), 120)], y_v[:, pl.ds(512, 128)], preferred_element_type=F32)
                  for u in range(4)]
            return jnp.concatenate([jnp.dot(wn, y_v[:, pl.ds(0, 512)], preferred_element_type=F32),
                                    jnp.concatenate(c4, axis=0)], axis=1)

        def abuild(C):
            C = C.reshape(5, 3, 8, D)
            B1 = C[0]
            for g in range(1, 5):
                B1 = jnp.where((cg == g)[None], C[g], B1)
            As = []
            for t in range(5):
                b1 = B1[:, :, 128 * t:128 * (t + 1)]
                b20 = b1.reshape(24, 128)[:DH]
                wp_v[t, pl.ds(0, DH, stride=2), :] = b20
                wp_v[t, pl.ds(1, DH, stride=2), :] = b20
                b2 = wp_v[t].reshape(5, 8, 128)
                hpt = hp[:, 128 * t:128 * (t + 1)]
                cht = ch[:, 128 * t:128 * (t + 1)]
                rows = []
                for u in range(4):
                    h0 = 2 * (3 * t + u)
                    if 3 * t + u in MIDS:
                        rows += [jnp.where((cht == h)[None], b1[:2], 0.0) for h in (h0, h0 + 1)
                                 if DH * h < 128 * (t + 1) and DH * (h + 1) > 128 * t]
                        rows.append(jnp.where((hpt == h0)[None], b2[4:], 0.0))
                    else:
                        rows.append(jnp.where((hpt == h0)[None], b2, 0.0))
                As.append(jnp.concatenate(rows, axis=0).reshape(-1, 128).astype(BF))
            return As

        done = [0] * (S // 128)
        nl = nt_ = nk = na = 0
        kvs, phiks, As = None, {}, None
        for g, (pieces, lns, units) in enumerate(PRO):
            with jax.named_scope(f"w_{g}"):
                for cp in groups[g]:
                    cp.wait()
            if g == 0:
                for cp in groups[-1]:
                    cp.start()
            if g == len(PRO) - 1:
                wstart()
            acc, nl0 = {}, nl
            news = sum(n for kind, n in pieces if kind == "k")
            for u in units:
                if u == "T":
                    for k in range(nt_, nt_ + news):
                        transpose_v(k)
                    nt_ += news
                    for c in range(nl, nl0 + lns):
                        lnt(c)
                    nl = max(nl, nl0 + lns)
                elif u == "C":
                    C = cmat()
                elif u in ("k", "q"):
                    As = As or abuild(C)
                    fold(As, 1 if u == "k" else 0)
                elif u == "K":
                    phiks[nk] = feats(1, TA * nk, TA)
                    nk += 1
                elif u == "A":
                    assert all(d == 5 for d in done[4 * na:4 * na + 4])
                    kvs = astep(kvs, na, phiks.pop(na))
                    na += 1
                elif u[0] == "N":
                    _, c0, nt, k, n, ns = u
                    for c in range(nl, c0 + nt):
                        lnt(c)
                    nl = max(nl, c0 + nt)
                    r = ndot(c0, nt, k, n, ns)
                    assert all(d == k for d in done[c0:c0 + nt])
                    if k:
                        r = r + vn_v[pl.ds(128 * c0, 128 * nt), :]
                    vn_v[pl.ds(128 * c0, 128 * nt), :] = r
                    done[c0:c0 + nt] = [k + n if k + n < 5 else -1] * nt
                elif u[0] == "X":
                    assert done[u[1]] == -1
                    vstore(vn_v[pl.ds(128 * u[1], 128), :].T, 128 * u[1], 128)
                    done[u[1]] = 5
                else:
                    c0, nt, k, n = u if len(u) == 4 else (u[0], 1, 0, 5)
                    for c in range(nl, c0 + nt):
                        lnt(c)
                    nl = max(nl, c0 + nt)
                    r = vdot(c0, nt, k, n)
                    for c in range(c0, c0 + nt):
                        rc = r[:, 128 * (c - c0):128 * (c - c0 + 1)]
                        if done[c]:
                            rc = rc + (acc[c] if c in acc else va_v[:, pl.ds(128 * (c % 5), 128)])
                        done[c] += n
                        acc[c] = rc
                        if done[c] == 5:
                            vstore(acc.pop(c), 128 * c, 128)
            for c, rc in acc.items():
                va_v[:, pl.ds(128 * (c % 5), 128)] = rc
        assert nl == S // 128 and nk == na == S // TA
        for g in range(NG - 1):
            kvb_v[g] = jnp.where(mk_v[g % 2] == 0, kvs[g], 0.0).astype(BF)
        kvl_v[...] = jnp.where(mk_v[2, pl.ds(0, 48), pl.ds(0, 2 * PR)] == 0, kvs[NG - 1], 0.0).astype(BF)
        with jax.named_scope("w_w"):
            cp_wo.wait(); cp_w1.wait(); cp_w3.wait(); cp_w2.wait()

    def attn(phiq):
        low = lax.broadcasted_iota(jnp.int32, (8, SB), 0) < 4
        ots = []
        for q in range(NS):
            n1 = jnp.dot(kvb_v[2 * q], phiq[2 * q], preferred_element_type=F32)
            n2 = jnp.dot(kvb_v[2 * q + 1], phiq[2 * q + 1], preferred_element_type=F32)
            r = _rcp(jnp.where(low, n2[:8], n1[56:]) + 1e-6)
            ra, rb, rc, rd, re, rf = [jnp.broadcast_to(r[k:k + 1], (8, SB)) for k in (4, 5, 6, 0, 1, 2)]
            num = jnp.concatenate([n1[:56], jnp.where(low, n1[56:], n2[:8]), n2[8:]], axis=0)
            scale = jnp.concatenate([ra, ra, jnp.where(low, ra, rb), rb, rb, rc, rc, jnp.where(low, rc, rd),
                                     rd, rd, re, re, jnp.where(low, re, rf), rf, rf], axis=0)
            ots.append(num * scale)
        ots = [ots[-1][:2 * PR]] + ots[:-1] + [ots[-1][2 * PR:]]
        nd = jnp.dot(kvl_v[...], phiq[NG - 1], preferred_element_type=F32)
        r = _rcp(nd[PR:PR + 8] + 1e-6)
        rs = pltpu.roll(r, 4, 0)
        ra = jnp.where(low, r, rs)
        rb = jnp.where(low, rs, r)
        ots.append(nd[:PR] * jnp.concatenate([ra, ra, r, rb, rb], axis=0))
        return jnp.concatenate(ots, axis=0).T

    def oproj(row, o):
        hs, hns = [], []
        m = SB // WP
        for u in range(WP):
            rw = pl.multiple_of(row + m * u, m)
            h = x_v[pl.ds(rw, m), :].astype(F32) + jnp.dot(o[m * u:m * (u + 1)].astype(BF), wo_v[...], preferred_element_type=F32)
            hs.append(h)
            hns.append(_ln(h).astype(BF))
        return jnp.concatenate(hs, axis=0), jnp.concatenate(hns, axis=0)

    def ffn(h, hn, row, splits):
        acc = h
        nc = F // FC
        for c in range(nc):
            gate = jnp.dot(hn, w1_v[:, pl.ds(FC * c, FC)], preferred_element_type=F32)
            up = jnp.dot(hn, w3_v[:, pl.ds(FC * c, FC)], preferred_element_type=F32)
            hg = 0.5 * gate
            act = (hg + hg * jnp.tanh(hg)) * up
            if c + 1 < nc:
                acc = acc + jnp.dot(act.astype(BF), w2_v[pl.ds(FC * c, FC), :], preferred_element_type=F32)
        r0 = 0
        for n, cols in splits:
            rw = pl.multiple_of(row + r0, 64)
            c0 = 0
            a = act[r0:r0 + n].astype(BF)
            for nc in cols:
                res = acc[r0:r0 + n, c0:c0 + nc] + jnp.dot(a, w2_v[pl.ds(F - FC, FC), pl.ds(c0, nc)],
                                                           preferred_element_type=F32)
                out_v[pl.ds(rw, n), pl.ds(c0, nc)] = res.astype(BF)
                ocopy(rw, n, c0, nc).start()
                c0 += nc
            r0 += n

    nsub = TB // SB
    splits = [((SB, (D,)),)] * (nsub - 1) + [OSPLIT]

    def body_b(j, carry):
        rows = [pl.multiple_of(j * TB + s * SB, SB) for s in range(nsub)]
        qs, os_, hs, nf = [], [], [], 0
        for o in ORB:
            if o == "Q":
                qs.append(feats(0, rows[len(qs)], SB))
            elif o == "A":
                os_.append(attn(qs[len(os_)]))
            elif o == "W":
                hs.append(oproj(rows[len(hs)], os_[len(hs)]))
            else:
                ffn(*hs[nf], rows[nf], splits[nf])
                nf += 1
        assert nf == nsub
        return carry

    with jax.named_scope("phaseB"):
        lax.fori_loop(0, NB, body_b, 0)

    with jax.named_scope("tail"):
        for j in range(NB):
            r0 = j * TB
            for sp in splits:
                for n, cols in sp:
                    c0 = 0
                    for nc in cols:
                        ocopy(r0, n, c0, nc).wait()
                        c0 += nc
                    r0 += n


def _full(c0, c1):
    return [(c,) for c in range(c0, c1)]


_PRO = [([("x", 3)], 2, ["T"]),
        ([("k", 1)], 1, [("N", 0, 3, 0, 1, 4), "T"]),
        ([("k", 2)], 0, [("N", 0, 3, 1, 2, 2), "T"]),
        ([("k", 2), ("x", 2)], 2, [("N", 0, 3, 3, 2, 2), "T", (3,), (4, 1, 0, 2)]),
        ([("x", 6)], 0, [(4, 1, 2, 3), ("X", 0), ("X", 1), ("X", 2)] + _full(5, 9) + [(9, 1, 0, 3), (10, 1, 0, 2)]),
        ([("p", 0), ("w", 0), ("x", 5)], 0,
         [(9, 1, 3, 2), "C", (10, 1, 2, 3), "k", (11,), "q"] + _full(12, 16) + list("KKAAKKAA"))]


def build(A_x, A_wqkv, A_w_phi, A_wo, B_x, B_w1, B_w3, B_w2, TA=512, TB=512, SB=256, FC=512,
          ORB="QQAAWWFF", WP=4, PRO=_PRO, OSPLIT=((128, (D,)), (64, (D,)), (64, (384, 128, 128)))):
    x2 = A_x.reshape(S, D)
    wphi_t = A_w_phi.transpose(1, 2, 0)
    any_spec = pl.BlockSpec(memory_space=pl.ANY)
    out = pl.pallas_call(
        functools.partial(_kernel, TA=TA, TB=TB, SB=SB, FC=FC, OSPLIT=OSPLIT, ORB=ORB, WP=WP, PRO=PRO),
        in_specs=[any_spec] * 7,
        out_specs=any_spec,
        out_shape=jax.ShapeDtypeStruct((S, D), BF),
        scratch_shapes=[
            pltpu.VMEM((S, D), BF),
            pltpu.VMEM((S, D), BF),
            pltpu.VMEM((S, D), BF),
            pltpu.VMEM((NG, 64, S), BF),
            pltpu.VMEM((DH, DH, H), BF),
            pltpu.VMEM((D, 3 * D), BF),
            pltpu.VMEM((D, D), BF),
            pltpu.VMEM((D, F), BF),
            pltpu.VMEM((D, F), BF),
            pltpu.VMEM((F, D), BF),
            pltpu.VMEM((3 * D, D), BF),
            pltpu.VMEM((5, PR, 128), F32),
            pltpu.VMEM((5, 24, 128), F32),
            pltpu.VMEM((128, D), BF),
            pltpu.VMEM((NG - 1, 64, 128), BF),
            pltpu.VMEM((48, 2 * PR), BF),
            pltpu.VMEM((3, 64, 128), jnp.int32),
            pltpu.VMEM((D, 640), F32),
            pltpu.VMEM((384, D), F32),
            pltpu.SemaphoreType.DMA((len(PRO) - 1,)),
        ],
        compiler_params=pltpu.CompilerParams(
            vmem_limit_bytes=100 * 1024 * 1024,
            disable_bounds_checks=True,
        ),
    )(x2, A_wqkv, wphi_t, A_wo, B_w1, B_w3, B_w2)
    return out.reshape(1, S, D)


@jax.jit
def pallas_sequential_preLN__linear_kernel_hedgehog__glu_gated_swiglu__prompt_kernel(
        A_x, A_wqkv, A_w_phi, A_wo, B_x, B_w1, B_w3, B_w2):
    return build(A_x, A_wqkv, A_w_phi, A_wo, B_x, B_w1, B_w3, B_w2)
```

```python
import functools
import math
import jax
import jax.numpy as jnp
from jax import lax
import jax.experimental.pallas as pl
import jax.experimental.pallas.tpu as pltpu

S, D, H, DH, F = 2048, 640, 32, 20, 1536
PR = 2 * DH
NS = 5
NG = 2 * NS + 1
SEXT = ((2, 3, 4), (5, 6, 7), (8, 9, 10), (11, 12, 13), (0, 1, 14))
MIDS = tuple(m for _, m, _ in SEXT)
NT_DIMS = (((1,), (1,)), ((), ()))
BF = jnp.bfloat16
F32 = jnp.float32
EPS = 1e-5
LOG2E = 1.4426950408889634


def _rcp(x):
    r = pl.reciprocal(x, approx=True)
    return r * (2.0 - x * r)


def _ln(x):
    m = jnp.mean(x, axis=-1, keepdims=True)
    xc = x - m
    v = jnp.mean(xc * xc, axis=-1, keepdims=True)
    return xc * lax.rsqrt(v + EPS)


def _red(x3, op):
    r = op(op(op(x3[0], x3[1]), op(x3[2], x3[3])), x3[4])
    r = op(r, pltpu.roll(r, 2, 0))
    r = op(r, pltpu.roll(r, 4, 0))
    return r


def _feat(p, T):
    p3 = p.reshape(5, 8, T)
    mx = _red(p3, jnp.maximum)
    mn = _red(p3, jnp.minimum)
    ep = jnp.exp2(p3 - mx[None])
    en = jnp.exp2(mn[None] - p3)
    rp = _rcp(_red(ep, jnp.add))
    rn = _rcp(_red(en, jnp.add))
    phi = jnp.concatenate([ep * rp[None], en * rn[None]], axis=0)
    return phi.reshape(2 * PR, T)


def _feat_split(p, T):
    even = lax.broadcasted_iota(jnp.int32, (8, T), 0) % 2 == 0

    def red(x3, op):
        m0, m1 = op(x3[0], x3[1]), op(x3[2], x3[3])
        r = op(op(jnp.where(even, m0, m1), pltpu.roll(jnp.where(even, m1, m0), 1, 0)), x3[4])
        r = op(r, pltpu.roll(r, 2, 0))
        return op(r, pltpu.roll(r, 4, 0))

    def spread(r):
        rs = pltpu.roll(r, 1, 0)
        r0, r1 = jnp.where(even, r, rs), jnp.where(even, rs, r)
        return jnp.stack([r0, r0, r1, r1, r], axis=0)

    p3 = p.reshape(5, 8, T)
    ep = jnp.exp2(p3 - spread(red(p3, jnp.maximum)))
    en = jnp.exp2(spread(red(p3, jnp.minimum)) - p3)
    ep = ep * spread(_rcp(red(ep, jnp.add)))
    en = en * spread(_rcp(red(en, jnp.add)))
    out = [jnp.concatenate([ep[i:j], en[i:j]], axis=0) for i, j in ((0, 2), (2, 4), (4, 5))]
    return [o.reshape(-1, T) for o in out]


def _kernel(x_hbm, wqkv_hbm, wphi_hbm, wo_hbm, w1_hbm, w3_hbm, w2_hbm, out_hbm,
            x_v, out_v, xn_v, vt_v, wphi_v, wqkv_v, wo_v, w1_v, w3_v, w2_v, wt_v, wp_v, wn_v, y_v, kvb_v, kvl_v, mk_v, va_v, vn_v, as_v,
            sems, *, TA, TB, SB, FC, OSPLIT, ORB, WP, PRO):
    NB = S // TB

    def wcopy(c0, n, sem):
        return pltpu.make_async_copy(wqkv_hbm.at[:, pl.ds(c0, n)], wqkv_v.at[:, pl.ds(c0, n)], sems.at[sem])

    def xcopy(r0, r1, sem):
        return pltpu.make_async_copy(x_hbm.at[pl.ds(r0, r1 - r0)], x_v.at[pl.ds(r0, r1 - r0)], sems.at[sem])

    def ocopy(r, n, c0=0, nc=D):
        return pltpu.make_async_copy(out_v.at[pl.ds(r, n), pl.ds(c0, nc)], out_hbm.at[pl.ds(r, n), pl.ds(c0, nc)],
                                     sems.at[1])

    def vcopy(r0, n, sem):
        return pltpu.make_async_copy(wqkv_hbm.at[pl.ds(r0, n), pl.ds(2 * D, D)],
                                     wqkv_v.at[pl.ds(r0, n), pl.ds(2 * D, D)], sems.at[sem])

    groups, nx, nk = [], 0, 0
    for g, (pieces, _, _) in enumerate(PRO):
        cps, sem = [], g % (len(PRO) - 1)
        for kind, n in pieces:
            if kind == "x":
                cps.append(xcopy(128 * nx, 128 * (nx + n), sem))
                nx += n
            elif kind == "k":
                cps.append(vcopy(128 * nk, 128 * n, sem))
                nk += n
            elif kind == "p":
                cps.append(pltpu.make_async_copy(wphi_hbm, wphi_v, sems.at[sem]))
            else:
                cps.append(wcopy(0, 2 * D, sem))
        groups.append(cps)
    assert nk == 5 and 128 * nx == S
    cp_wo = pltpu.make_async_copy(wo_hbm, wo_v, sems.at[1])
    cp_w1 = pltpu.make_async_copy(w1_hbm, w1_v, sems.at[1])
    cp_w3 = pltpu.make_async_copy(w3_hbm, w3_v, sems.at[1])
    cp_w2 = pltpu.make_async_copy(w2_hbm, w2_v, sems.at[1])

    def wstart():
        cp_wo.start(); cp_w1.start(); cp_w3.start(); cp_w2.start()

    def dot2(w, xn, ms=None):
        tiles = (xn.shape[0] // 128) * (xn.shape[1] // 128)
        ns = 4 // math.gcd(4, tiles)
        ms = ms or [w.shape[0] // ns] * ns
        return jnp.concatenate([lax.dot_general(w[sum(ms[:u]):sum(ms[:u + 1])], xn, NT_DIMS,
                                                preferred_element_type=F32) for u in range(len(ms))], axis=0)

    def vstore(pv, c0, n):
        low = lax.broadcasted_iota(jnp.int32, (8, n), 0) < 4
        for q, (a, m, c) in enumerate(SEXT):
            r = PR * m
            mid = pv[r + 16:r + 24]
            vt_v[2 * q, :, pl.ds(c0, n)] = jnp.concatenate(
                [pv[PR * a:PR * (a + 1)], pv[r:r + 16], jnp.where(low, mid, 1.0)], axis=0).astype(BF)
            vt_v[2 * q + 1, :, pl.ds(c0, n)] = jnp.concatenate(
                [jnp.where(low, 1.0, mid), pv[r + 24:r + PR], pv[PR * c:PR * (c + 1)]], axis=0).astype(BF)
        vt_v[NG - 1, pl.ds(0, 48), pl.ds(c0, n)] = jnp.concatenate(
            [pv[D - PR:], jnp.ones((8, n), F32)], axis=0).astype(BF)

    def transpose_v(k):
        wt_v[pl.ds(2 * D, D), pl.ds(128 * k, 128)] = (
            wqkv_v[pl.ds(128 * k, 128), pl.ds(2 * D, D)].astype(F32).T.astype(BF))

    def vdot(c, nt, k, nk):
        return dot2(wt_v[pl.ds(2 * D, D), pl.ds(128 * k, 128 * nk)],
                    xn_v[pl.ds(128 * c, 128 * nt), pl.ds(128 * k, 128 * nk)])

    def ndot(c, nt, k, nk, ns):
        m = 128 * nt // ns
        return jnp.concatenate([jnp.dot(xn_v[pl.ds(128 * c + m * u, m), pl.ds(128 * k, 128 * nk)],
                                        wqkv_v[pl.ds(128 * k, 128 * nk), pl.ds(2 * D, D)],
                                        preferred_element_type=F32) for u in range(ns)], axis=0)

    def fold(As, s):
        prev = None
        for t in range(5):
            w = wqkv_v[:, pl.ds(D * s + 128 * t, 128)]
            res = dot2(As[t][...], w, [80, 80] if (s, t) == (1, 2) else [As[t].shape[0]])
            if t in (1, 2):
                res = jnp.concatenate([res[:16] + prev[:16], res[16:32], res[32:PR] + prev[16:], res[PR:]], axis=0)
            elif t > 2:
                res = jnp.concatenate([prev[:16], prev[16:] + res[:24], res[24:]], axis=0)
            n = 160 if t == 4 else 120
            wt_v[pl.ds(D * s + 120 * t, n), :] = (res[:n] * LOG2E).astype(BF)
            prev = res[120:]

    def feats(s, row, n):
        pk = dot2(wt_v[pl.ds(D * s, D), :], xn_v[pl.ds(row, n), :])
        out = []
        for a, m, c in SEXT:
            fa = _feat(pk[PR * a:PR * (a + 1)], n)
            f0, f1, fm = _feat_split(pk[PR * m:PR * (m + 1)], n)
            fc = _feat(pk[PR * c:PR * (c + 1)], n)
            out += [jnp.concatenate([fa, f0, fm], axis=0).astype(BF), jnp.concatenate([fc, f1, fm], axis=0).astype(BF)]
        return out + [_feat(pk[D - PR:], n).astype(BF)]

    def astep(kvs, b, phiks):
        out = []
        for g in range(NG):
            m = 64 if g < NG - 1 else 48
            kv = lax.dot_general(vt_v[g, pl.ds(0, m), pl.ds(TA * b, TA)], phiks[g], NT_DIMS,
                                 preferred_element_type=F32)
            out.append(kv if kvs is None else kv + kvs[g])
        return out

    def lnt(c, n=128):
        xn_v[pl.ds(128 * c, n), :] = _ln(x_v[pl.ds(128 * c, n), :].astype(F32)).astype(BF)

    with jax.named_scope("prologue"):
        for cps in groups[:-1]:
            for cp in cps:
                cp.start()

        c8 = lax.broadcasted_iota(jnp.int32, (8, D), 1)
        r8 = lax.broadcasted_iota(jnp.int32, (8, D), 0)
        ch = c8 // DH
        hp = ch - r8 % 2
        wn_v[...] = jnp.zeros(wn_v.shape, F32)

        rr = lax.broadcasted_iota(jnp.int32, (64, 128), 0)
        cc = lax.broadcasted_iota(jnp.int32, (64, 128), 1)
        par = cc % 2
        for e in range(2):
            head_c = jnp.where(cc < 2 * PR, par, jnp.where((cc < 112) | (par == e), 2, 3))
            if e == 0:
                head_r = jnp.where(rr < 60, rr // DH, jnp.minimum(rr - 60, 2))
            else:
                head_r = (jnp.where(rr < 4, jnp.minimum(rr, 2), (rr - 4) // DH) + 2) % 3
            mk_v[e] = head_r - head_c
        mk_v[2] = jnp.where(rr < PR, rr // DH, (rr - PR) // 4) - par

        def cmat():
            w = wphi_v[...].astype(F32)
            for g in range(5):
                wn_v[g, pl.ds(0, DH), :] = jnp.concatenate([w[4 * g + l] for l in range(4)], axis=1)
                wg = wn_v[g].T
                for l in range(4):
                    y_v[pl.ds(4 * g + l, H, stride=DH), :] = wg[H * l:H * (l + 1)]
            return y_v[...].T[:24]

        def abuild(C):
            B1 = C.reshape(3, 8, D)
            As = []
            for t in range(5):
                b1 = B1[:, :, 128 * t:128 * (t + 1)]
                b20 = b1.reshape(24, 128)[:DH]
                wp_v[t, pl.ds(0, DH, stride=2), :] = b20
                wp_v[t, pl.ds(1, DH, stride=2), :] = b20
                b2 = wp_v[t].reshape(5, 8, 128)
                hpt = hp[:, 128 * t:128 * (t + 1)]
                cht = ch[:, 128 * t:128 * (t + 1)]
                rows = []
                for u in range(4):
                    h0 = 2 * (3 * t + u)
                    if 3 * t + u in MIDS:
                        rows += [jnp.where((cht == h)[None], b1[:2], 0.0) for h in (h0, h0 + 1)
                                 if DH * h < 128 * (t + 1) and DH * (h + 1) > 128 * t]
                        rows.append(jnp.where((hpt == h0)[None], b2[4:], 0.0))
                    else:
                        rows.append(jnp.where((hpt == h0)[None], b2, 0.0))
                As.append(jnp.concatenate(rows, axis=0).reshape(-1, 128).astype(BF))
            return As

        done = [0] * (S // 128)
        nl = nt_ = nk = na = 0
        kvs, phiks, As = None, {}, None
        for g, (pieces, lns, units) in enumerate(PRO):
            with jax.named_scope(f"w_{g}"):
                for cp in groups[g]:
                    cp.wait()
            if g == 0:
                for cp in groups[-1]:
                    cp.start()
            if g == len(PRO) - 1:
                wstart()
            acc, nl0 = {}, nl
            news = sum(n for kind, n in pieces if kind == "k")
            for u in units:
                if u == "T":
                    for k in range(nt_, nt_ + news):
                        transpose_v(k)
                    nt_ += news
                    for c in range(nl, nl0 + lns):
                        lnt(c)
                    nl = max(nl, nl0 + lns)
                elif u == "B":
                    for t, a in enumerate(abuild(cmat())):
                        as_v[t, pl.ds(0, a.shape[0]), :] = a
                    As = [as_v.at[t, pl.ds(0, 160 if t == 2 else 144), :] for t in range(5)]
                elif u in ("k", "q"):
                    fold(As, 1 if u == "k" else 0)
                elif u == "K":
                    phiks[nk] = feats(1, TA * nk, TA)
                    nk += 1
                elif u == "A":
                    assert all(d == 5 for d in done[4 * na:4 * na + 4])
                    kvs = astep(kvs, na, phiks.pop(na))
                    na += 1
                elif u[0] == "N":
                    _, c0, nt, k, n, ns = u
                    for c in range(nl, c0 + nt):
                        lnt(c)
                    nl = max(nl, c0 + nt)
                    r = ndot(c0, nt, k, n, ns)
                    assert all(d == k for d in done[c0:c0 + nt])
                    if k:
                        r = r + vn_v[pl.ds(128 * c0, 128 * nt), :]
                    vn_v[pl.ds(128 * c0, 128 * nt), :] = r
                    done[c0:c0 + nt] = [k + n if k + n < 5 else -1] * nt
                elif u[0] == "X":
                    assert done[u[1]] == -1
                    vstore(vn_v[pl.ds(128 * u[1], 128), :].T, 128 * u[1], 128)
                    done[u[1]] = 5
                else:
                    c0, nt, k, n = u if len(u) == 4 else (u[0], 1, 0, 5)
                    for c in range(nl, c0 + nt):
                        lnt(c)
                    nl = max(nl, c0 + nt)
                    r = vdot(c0, nt, k, n)
                    for c in range(c0, c0 + nt):
                        rc = r[:, 128 * (c - c0):128 * (c - c0 + 1)]
                        if done[c]:
                            rc = rc + (acc[c] if c in acc else va_v[...])
                        done[c] += n
                        acc[c] = rc
                        if done[c] == 5:
                            vstore(acc.pop(c), 128 * c, 128)
            assert len(acc) <= 1
            for rc in acc.values():
                va_v[...] = rc
        assert nl == S // 128 and nk == na == S // TA
        for g in range(NG - 1):
            kvb_v[g] = jnp.where(mk_v[g % 2] == 0, kvs[g], 0.0).astype(BF)
        kvl_v[...] = jnp.where(mk_v[2, pl.ds(0, 48), pl.ds(0, 2 * PR)] == 0, kvs[NG - 1], 0.0).astype(BF)
        with jax.named_scope("w_w"):
            cp_wo.wait(); cp_w1.wait(); cp_w3.wait(); cp_w2.wait()

    def attn(phiq):
        low = lax.broadcasted_iota(jnp.int32, (8, SB), 0) < 4
        ots = []
        for q in range(NS):
            n1 = jnp.dot(kvb_v[2 * q], phiq[2 * q], preferred_element_type=F32)
            n2 = jnp.dot(kvb_v[2 * q + 1], phiq[2 * q + 1], preferred_element_type=F32)
            r = _rcp(jnp.where(low, n2[:8], n1[56:]) + 1e-6)
            ra, rb, rc, rd, re, rf = [jnp.broadcast_to(r[k:k + 1], (8, SB)) for k in (4, 5, 6, 0, 1, 2)]
            num = jnp.concatenate([n1[:56], jnp.where(low, n1[56:], n2[:8]), n2[8:]], axis=0)
            scale = jnp.concatenate([ra, ra, jnp.where(low, ra, rb), rb, rb, rc, rc, jnp.where(low, rc, rd),
                                     rd, rd, re, re, jnp.where(low, re, rf), rf, rf], axis=0)
            ots.append(num * scale)
        ots = [ots[-1][:2 * PR]] + ots[:-1] + [ots[-1][2 * PR:]]
        nd = jnp.dot(kvl_v[...], phiq[NG - 1], preferred_element_type=F32)
        r = _rcp(nd[PR:PR + 8] + 1e-6)
        rs = pltpu.roll(r, 4, 0)
        ra = jnp.where(low, r, rs)
        rb = jnp.where(low, rs, r)
        ots.append(nd[:PR] * jnp.concatenate([ra, ra, r, rb, rb], axis=0))
        return jnp.concatenate(ots, axis=0).T

    def oproj(row, o):
        hs, hns = [], []
        m = SB // WP
        for u in range(WP):
            rw = pl.multiple_of(row + m * u, m)
            h = x_v[pl.ds(rw, m), :].astype(F32) + jnp.dot(o[m * u:m * (u + 1)].astype(BF), wo_v[...], preferred_element_type=F32)
            hs.append(h)
            hns.append(_ln(h).astype(BF))
        return jnp.concatenate(hs, axis=0), jnp.concatenate(hns, axis=0)

    def ffn(h, hn, row, splits):
        acc = h
        nc = F // FC
        for c in range(nc):
            gate = jnp.dot(hn, w1_v[:, pl.ds(FC * c, FC)], preferred_element_type=F32)
            up = jnp.dot(hn, w3_v[:, pl.ds(FC * c, FC)], preferred_element_type=F32)
            hg = 0.5 * gate
            act = (hg + hg * jnp.tanh(hg)) * up
            if c + 1 < nc:
                acc = acc + jnp.dot(act.astype(BF), w2_v[pl.ds(FC * c, FC), :], preferred_element_type=F32)
        r0 = 0
        for n, cols in splits:
            rw = pl.multiple_of(row + r0, 64)
            c0 = 0
            a = act[r0:r0 + n].astype(BF)
            for nc in cols:
                res = acc[r0:r0 + n, c0:c0 + nc] + jnp.dot(a, w2_v[pl.ds(F - FC, FC), pl.ds(c0, nc)],
                                                           preferred_element_type=F32)
                out_v[pl.ds(rw, n), pl.ds(c0, nc)] = res.astype(BF)
                ocopy(rw, n, c0, nc).start()
                c0 += nc
            r0 += n

    nsub = TB // SB
    splits = [((SB, (D,)),)] * (nsub - 1) + [OSPLIT]

    def body_b(j, carry):
        rows = [pl.multiple_of(j * TB + s * SB, SB) for s in range(nsub)]
        qs, os_, hs, nf = [], [], [], 0
        for o in ORB:
            if o == "Q":
                qs.append(feats(0, rows[len(qs)], SB))
            elif o == "A":
                os_.append(attn(qs[len(os_)]))
            elif o == "W":
                hs.append(oproj(rows[len(hs)], os_[len(hs)]))
            else:
                ffn(*hs[nf], rows[nf], splits[nf])
                nf += 1
        assert nf == nsub
        return carry

    with jax.named_scope("phaseB"):
        lax.fori_loop(0, NB, body_b, 0)

    with jax.named_scope("tail"):
        for j in range(NB):
            r0 = j * TB
            for sp in splits:
                for n, cols in sp:
                    c0 = 0
                    for nc in cols:
                        ocopy(r0, n, c0, nc).wait()
                        c0 += nc
                    r0 += n


def _full(c0, c1):
    return [(c,) for c in range(c0, c1)]


_PRO = [([("x", 3)], 2, ["T"]),
        ([("k", 1)], 1, [("N", 0, 3, 0, 1, 4), "T"]),
        ([("k", 2)], 0, [("N", 0, 3, 1, 2, 2), "T"]),
        ([("k", 2), ("x", 2)], 2, [("N", 0, 3, 3, 2, 2), "T", (3,), (4, 1, 0, 2)]),
        ([("x", 6), ("p", 0)], 0, [(4, 1, 2, 3), (5,), ("X", 0), (6,), ("X", 1), (7,), "B", ("X", 2)] + _full(8, 11)),
        ([("w", 0), ("x", 5)], 0, ["k", "q"] + _full(11, 16) + list("KKAAKKAA"))]


def build(A_x, A_wqkv, A_w_phi, A_wo, B_x, B_w1, B_w3, B_w2, TA=512, TB=512, SB=256, FC=512,
          ORB="QQAAWWFF", WP=4, PRO=_PRO, OSPLIT=((128, (D,)), (64, (D,)), (64, (384, 128, 128)))):
    x2 = A_x.reshape(S, D)
    wphi_t = A_w_phi.transpose(1, 2, 0)
    any_spec = pl.BlockSpec(memory_space=pl.ANY)
    out = pl.pallas_call(
        functools.partial(_kernel, TA=TA, TB=TB, SB=SB, FC=FC, OSPLIT=OSPLIT, ORB=ORB, WP=WP, PRO=PRO),
        in_specs=[any_spec] * 7,
        out_specs=any_spec,
        out_shape=jax.ShapeDtypeStruct((S, D), BF),
        scratch_shapes=[
            pltpu.VMEM((S, D), BF),
            pltpu.VMEM((S, D), BF),
            pltpu.VMEM((S, D), BF),
            pltpu.VMEM((NG, 64, S), BF),
            pltpu.VMEM((DH, DH, H), BF),
            pltpu.VMEM((D, 3 * D), BF),
            pltpu.VMEM((D, D), BF),
            pltpu.VMEM((D, F), BF),
            pltpu.VMEM((D, F), BF),
            pltpu.VMEM((F, D), BF),
            pltpu.VMEM((3 * D, D), BF),
            pltpu.VMEM((5, PR, 128), F32),
            pltpu.VMEM((5, 128, 128), F32),
            pltpu.VMEM((D, 128), F32),
            pltpu.VMEM((NG - 1, 64, 128), BF),
            pltpu.VMEM((48, 2 * PR), BF),
            pltpu.VMEM((3, 64, 128), jnp.int32),
            pltpu.VMEM((D, 128), F32),
            pltpu.VMEM((384, D), F32),
            pltpu.VMEM((5, 160, 128), BF),
            pltpu.SemaphoreType.DMA((len(PRO) - 1,)),
        ],
        compiler_params=pltpu.CompilerParams(
            vmem_limit_bytes=100 * 1024 * 1024,
            disable_bounds_checks=True,
        ),
    )(x2, A_wqkv, wphi_t, A_wo, B_w1, B_w3, B_w2)
    return out.reshape(1, S, D)


@jax.jit
def pallas_sequential_preLN__linear_kernel_hedgehog__glu_gated_swiglu__prompt_kernel(
        A_x, A_wqkv, A_w_phi, A_wo, B_x, B_w1, B_w3, B_w2):
    return build(A_x, A_wqkv, A_w_phi, A_wo, B_x, B_w1, B_w3, B_w2)
```

```python
import functools
import math
import jax
import jax.numpy as jnp
from jax import lax
import jax.experimental.pallas as pl
import jax.experimental.pallas.tpu as pltpu

S, D, H, DH, F = 2048, 640, 32, 20, 1536
PR = 2 * DH
NS = 5
NG = 2 * NS + 1
SEXT = ((2, 3, 4), (5, 6, 7), (8, 9, 10), (11, 12, 13), (0, 1, 14))
MIDS = tuple(m for _, m, _ in SEXT)
FC0 = (0, 80, 128, 240, 320, 384, 480, 512)
NT_DIMS = (((1,), (1,)), ((), ()))
BF = jnp.bfloat16
F32 = jnp.float32
EPS = 1e-5
LOG2E = 1.4426950408889634


def _rcp(x):
    r = pl.reciprocal(x, approx=True)
    return r * (2.0 - x * r)


def _ln(x):
    m = jnp.mean(x, axis=-1, keepdims=True)
    xc = x - m
    v = jnp.mean(xc * xc, axis=-1, keepdims=True)
    return xc * lax.rsqrt(v + EPS)


def _red(x3, op):
    r = op(op(op(x3[0], x3[1]), op(x3[2], x3[3])), x3[4])
    r = op(r, pltpu.roll(r, 2, 0))
    r = op(r, pltpu.roll(r, 4, 0))
    return r


def _feat(p, T):
    p3 = p.reshape(5, 8, T)
    mx = _red(p3, jnp.maximum)
    mn = _red(p3, jnp.minimum)
    ep = jnp.exp2(p3 - mx[None])
    en = jnp.exp2(mn[None] - p3)
    rp = _rcp(_red(ep, jnp.add))
    rn = _rcp(_red(en, jnp.add))
    phi = jnp.concatenate([ep * rp[None], en * rn[None]], axis=0)
    return phi.reshape(2 * PR, T)


def _feat_split(p, T):
    even = lax.broadcasted_iota(jnp.int32, (8, T), 0) % 2 == 0

    def red(x3, op):
        m0, m1 = op(x3[0], x3[1]), op(x3[2], x3[3])
        r = op(op(jnp.where(even, m0, m1), pltpu.roll(jnp.where(even, m1, m0), 1, 0)), x3[4])
        r = op(r, pltpu.roll(r, 2, 0))
        return op(r, pltpu.roll(r, 4, 0))

    def spread(r):
        rs = pltpu.roll(r, 1, 0)
        r0, r1 = jnp.where(even, r, rs), jnp.where(even, rs, r)
        return jnp.stack([r0, r0, r1, r1, r], axis=0)

    p3 = p.reshape(5, 8, T)
    ep = jnp.exp2(p3 - spread(red(p3, jnp.maximum)))
    en = jnp.exp2(spread(red(p3, jnp.minimum)) - p3)
    ep = ep * spread(_rcp(red(ep, jnp.add)))
    en = en * spread(_rcp(red(en, jnp.add)))
    out = [jnp.concatenate([ep[i:j], en[i:j]], axis=0) for i, j in ((0, 2), (2, 4), (4, 5))]
    return [o.reshape(-1, T) for o in out]


def _kernel(x_hbm, wqkv_hbm, wphi_hbm, wo_hbm, w1_hbm, w3_hbm, w2_hbm, out_hbm,
            x_v, out_v, xn_v, vt_v, wphi_v, wqkv_v, wo_v, w1_v, w3_v, w2_v, wt_v, wp_v, wn_v, y_v, kvb_v, kvl_v, mk_v, va_v, vn_v, as_v,
            sems, *, TA, TB, SB, FC, OSPLIT, ORB, WP, PRO):
    NB = S // TB

    def wcopy(c0, n, sem):
        return pltpu.make_async_copy(wqkv_hbm.at[:, pl.ds(c0, n)], wqkv_v.at[:, pl.ds(c0, n)], sems.at[sem])

    def xcopy(r0, r1, sem):
        return pltpu.make_async_copy(x_hbm.at[pl.ds(r0, r1 - r0)], x_v.at[pl.ds(r0, r1 - r0)], sems.at[sem])

    def ocopy(r, n, c0=0, nc=D):
        return pltpu.make_async_copy(out_v.at[pl.ds(r, n), pl.ds(c0, nc)], out_hbm.at[pl.ds(r, n), pl.ds(c0, nc)],
                                     sems.at[1])

    def vcopy(r0, n, sem):
        return pltpu.make_async_copy(wqkv_hbm.at[pl.ds(r0, n), pl.ds(2 * D, D)],
                                     wqkv_v.at[pl.ds(r0, n), pl.ds(2 * D, D)], sems.at[sem])

    groups, nx, nk = [], 0, 0
    for g, (pieces, _, _) in enumerate(PRO):
        cps, sem = [], g % (len(PRO) - 1)
        for kind, n in pieces:
            if kind == "x":
                cps.append(xcopy(128 * nx, 128 * (nx + n), sem))
                nx += n
            elif kind == "k":
                cps.append(vcopy(128 * nk, 128 * n, sem))
                nk += n
            elif kind == "p":
                cps.append(pltpu.make_async_copy(wphi_hbm, wphi_v, sems.at[sem]))
            else:
                cps.append(wcopy(0, 2 * D, sem))
        groups.append(cps)
    assert nk == 5 and 128 * nx == S
    cp_wo = pltpu.make_async_copy(wo_hbm, wo_v, sems.at[1])
    cp_w1 = pltpu.make_async_copy(w1_hbm, w1_v, sems.at[1])
    cp_w3 = pltpu.make_async_copy(w3_hbm, w3_v, sems.at[1])
    cp_w2 = pltpu.make_async_copy(w2_hbm, w2_v, sems.at[1])

    def wstart():
        cp_wo.start(); cp_w1.start(); cp_w3.start(); cp_w2.start()

    def dot2(w, xn, ms=None):
        tiles = (xn.shape[0] // 128) * (xn.shape[1] // 128)
        ns = 4 // math.gcd(4, tiles)
        ms = ms or [w.shape[0] // ns] * ns
        return jnp.concatenate([lax.dot_general(w[sum(ms[:u]):sum(ms[:u + 1])], xn, NT_DIMS,
                                                preferred_element_type=F32) for u in range(len(ms))], axis=0)

    def vstore(pv, c0, n):
        low = lax.broadcasted_iota(jnp.int32, (8, n), 0) < 4
        for q, (a, m, c) in enumerate(SEXT):
            r = PR * m
            mid = pv[r + 16:r + 24]
            vt_v[2 * q, :, pl.ds(c0, n)] = jnp.concatenate(
                [pv[PR * a:PR * (a + 1)], pv[r:r + 16], jnp.where(low, mid, 1.0)], axis=0).astype(BF)
            vt_v[2 * q + 1, :, pl.ds(c0, n)] = jnp.concatenate(
                [jnp.where(low, 1.0, mid), pv[r + 24:r + PR], pv[PR * c:PR * (c + 1)]], axis=0).astype(BF)
        vt_v[NG - 1, pl.ds(0, 48), pl.ds(c0, n)] = jnp.concatenate(
            [pv[D - PR:], jnp.ones((8, n), F32)], axis=0).astype(BF)

    def transpose_v(k):
        wt_v[pl.ds(2 * D, D), pl.ds(128 * k, 128)] = (
            wqkv_v[pl.ds(128 * k, 128), pl.ds(2 * D, D)].astype(F32).T.astype(BF))

    def vdot(c, nt, k, nk):
        return dot2(wt_v[pl.ds(2 * D, D), pl.ds(128 * k, 128 * nk)],
                    xn_v[pl.ds(128 * c, 128 * nt), pl.ds(128 * k, 128 * nk)])

    def ndot(c, nt, k, nk, ns):
        m = 128 * nt // ns
        return jnp.concatenate([jnp.dot(xn_v[pl.ds(128 * c + m * u, m), pl.ds(128 * k, 128 * nk)],
                                        wqkv_v[pl.ds(128 * k, 128 * nk), pl.ds(2 * D, D)],
                                        preferred_element_type=F32) for u in range(ns)], axis=0)

    def fold(As, s, gs):
        for g in gs:
            res = dot2(As[g][...], wqkv_v[:, pl.ds(D * s + FC0[g], 128)], [2 * PR])
            wt_v[pl.ds(D * s + 2 * PR * g, 2 * PR), :] = (res * LOG2E).astype(BF)

    def feats(s, row, n):
        pk = dot2(wt_v[pl.ds(D * s, D), :], xn_v[pl.ds(row, n), :])
        out = []
        for a, m, c in SEXT:
            fa = _feat(pk[PR * a:PR * (a + 1)], n)
            f0, f1, fm = _feat_split(pk[PR * m:PR * (m + 1)], n)
            fc = _feat(pk[PR * c:PR * (c + 1)], n)
            out += [jnp.concatenate([fa, f0, fm], axis=0).astype(BF), jnp.concatenate([fc, f1, fm], axis=0).astype(BF)]
        return out + [_feat(pk[D - PR:], n).astype(BF)]

    def astep(kvs, b, phiks):
        out = []
        for g in range(NG):
            m = 64 if g < NG - 1 else 48
            kv = lax.dot_general(vt_v[g, pl.ds(0, m), pl.ds(TA * b, TA)], phiks[g], NT_DIMS,
                                 preferred_element_type=F32)
            out.append(kv if kvs is None else kv + kvs[g])
        return out

    def lnt(c, n=128):
        xn_v[pl.ds(128 * c, n), :] = _ln(x_v[pl.ds(128 * c, n), :].astype(F32)).astype(BF)

    with jax.named_scope("prologue"):
        for cps in groups[:-1]:
            for cp in cps:
                cp.start()

        c8 = lax.broadcasted_iota(jnp.int32, (8, 128), 1)
        r8 = lax.broadcasted_iota(jnp.int32, (8, 128), 0)
        wn_v[...] = jnp.zeros(wn_v.shape, F32)

        rr = lax.broadcasted_iota(jnp.int32, (64, 128), 0)
        cc = lax.broadcasted_iota(jnp.int32, (64, 128), 1)
        par = cc % 2
        for e in range(2):
            head_c = jnp.where(cc < 2 * PR, par, jnp.where((cc < 112) | (par == e), 2, 3))
            if e == 0:
                head_r = jnp.where(rr < 60, rr // DH, jnp.minimum(rr - 60, 2))
            else:
                head_r = (jnp.where(rr < 4, jnp.minimum(rr, 2), (rr - 4) // DH) + 2) % 3
            mk_v[e] = head_r - head_c
        mk_v[2] = jnp.where(rr < PR, rr // DH, (rr - PR) // 4) - par

        def cmat():
            w = wphi_v[...].astype(F32)
            for g in range(5):
                wn_v[g, pl.ds(0, DH), :] = jnp.concatenate([w[4 * g + l] for l in range(4)], axis=1)
                wg = wn_v[g].T
                for l in range(4):
                    y_v[pl.ds(4 * g + l, H, stride=DH), :] = wg[H * l:H * (l + 1)]
            return y_v[...].T[:24]

        def abuild(C):
            B1 = C.reshape(3, 8, D)
            As = []
            for g, c0 in enumerate(FC0):
                b1 = B1[:, :, c0:c0 + 128]
                b20 = b1.reshape(24, 128)[:DH]
                wp_v[g, pl.ds(0, DH, stride=2), :] = b20
                wp_v[g, pl.ds(1, DH, stride=2), :] = b20
                b2 = wp_v[g].reshape(5, 8, 128)
                ch = (c8 + c0) // DH
                hp = ch - r8 % 2
                rows = []
                for p in (2 * g, 2 * g + 1):
                    if p in MIDS:
                        rows += [jnp.where((ch == h)[None], b1[:2], 0.0) for h in (2 * p, 2 * p + 1)]
                        rows.append(jnp.where((hp == 2 * p)[None], b2[4:], 0.0))
                    else:
                        rows.append(jnp.where((hp == 2 * p)[None], b2, 0.0))
                As.append(jnp.concatenate(rows, axis=0).reshape(2 * PR, 128).astype(BF))
            return As

        done = [0] * (S // 128)
        nl = nt_ = nk = na = 0
        kvs, phiks, As = None, {}, None
        for g, (pieces, lns, units) in enumerate(PRO):
            with jax.named_scope(f"w_{g}"):
                for cp in groups[g]:
                    cp.wait()
            if g == 0:
                for cp in groups[-1]:
                    cp.start()
            if g == len(PRO) - 1:
                wstart()
            acc, nl0 = {}, nl
            news = sum(n for kind, n in pieces if kind == "k")
            for u in units:
                if u == "T":
                    for k in range(nt_, nt_ + news):
                        transpose_v(k)
                    nt_ += news
                    for c in range(nl, nl0 + lns):
                        lnt(c)
                    nl = max(nl, nl0 + lns)
                elif u == "B":
                    for t, a in enumerate(abuild(cmat())):
                        as_v[t] = a
                    As = [as_v.at[t] for t in range(8)]
                elif u[0] in ("k", "q"):
                    fold(As, 1 if u[0] == "k" else 0, [int(g) for g in u[1:]])
                elif u == "K":
                    phiks[nk] = feats(1, TA * nk, TA)
                    nk += 1
                elif u == "A":
                    assert all(d == 5 for d in done[4 * na:4 * na + 4])
                    kvs = astep(kvs, na, phiks.pop(na))
                    na += 1
                elif u[0] == "N":
                    _, c0, nt, k, n, ns = u
                    for c in range(nl, c0 + nt):
                        lnt(c)
                    nl = max(nl, c0 + nt)
                    r = ndot(c0, nt, k, n, ns)
                    assert all(d == k for d in done[c0:c0 + nt])
                    if k:
                        r = r + vn_v[pl.ds(128 * c0, 128 * nt), :]
                    vn_v[pl.ds(128 * c0, 128 * nt), :] = r
                    done[c0:c0 + nt] = [k + n if k + n < 5 else -1] * nt
                elif u[0] == "X":
                    assert done[u[1]] == -1
                    vstore(vn_v[pl.ds(128 * u[1], 128), :].T, 128 * u[1], 128)
                    done[u[1]] = 5
                else:
                    c0, nt, k, n = u if len(u) == 4 else (u[0], 1, 0, 5)
                    for c in range(nl, c0 + nt):
                        lnt(c)
                    nl = max(nl, c0 + nt)
                    r = vdot(c0, nt, k, n)
                    for c in range(c0, c0 + nt):
                        rc = r[:, 128 * (c - c0):128 * (c - c0 + 1)]
                        if done[c]:
                            rc = rc + (acc[c] if c in acc else va_v[...])
                        done[c] += n
                        acc[c] = rc
                        if done[c] == 5:
                            vstore(acc.pop(c), 128 * c, 128)
            assert len(acc) <= 1
            for rc in acc.values():
                va_v[...] = rc
        assert nl == S // 128 and nk == na == S // TA
        for g in range(NG - 1):
            kvb_v[g] = jnp.where(mk_v[g % 2] == 0, kvs[g], 0.0).astype(BF)
        kvl_v[...] = jnp.where(mk_v[2, pl.ds(0, 48), pl.ds(0, 2 * PR)] == 0, kvs[NG - 1], 0.0).astype(BF)
        with jax.named_scope("w_w"):
            cp_wo.wait(); cp_w1.wait(); cp_w3.wait(); cp_w2.wait()

    def attn(phiq):
        low = lax.broadcasted_iota(jnp.int32, (8, SB), 0) < 4
        ots = []
        for q in range(NS):
            n1 = jnp.dot(kvb_v[2 * q], phiq[2 * q], preferred_element_type=F32)
            n2 = jnp.dot(kvb_v[2 * q + 1], phiq[2 * q + 1], preferred_element_type=F32)
            r = _rcp(jnp.where(low, n2[:8], n1[56:]) + 1e-6)
            ra, rb, rc, rd, re, rf = [jnp.broadcast_to(r[k:k + 1], (8, SB)) for k in (4, 5, 6, 0, 1, 2)]
            num = jnp.concatenate([n1[:56], jnp.where(low, n1[56:], n2[:8]), n2[8:]], axis=0)
            scale = jnp.concatenate([ra, ra, jnp.where(low, ra, rb), rb, rb, rc, rc, jnp.where(low, rc, rd),
                                     rd, rd, re, re, jnp.where(low, re, rf), rf, rf], axis=0)
            ots.append(num * scale)
        ots = [ots[-1][:2 * PR]] + ots[:-1] + [ots[-1][2 * PR:]]
        nd = jnp.dot(kvl_v[...], phiq[NG - 1], preferred_element_type=F32)
        r = _rcp(nd[PR:PR + 8] + 1e-6)
        rs = pltpu.roll(r, 4, 0)
        ra = jnp.where(low, r, rs)
        rb = jnp.where(low, rs, r)
        ots.append(nd[:PR] * jnp.concatenate([ra, ra, r, rb, rb], axis=0))
        return jnp.concatenate(ots, axis=0).T

    def oproj(row, o):
        hs, hns = [], []
        m = SB // WP
        for u in range(WP):
            rw = pl.multiple_of(row + m * u, m)
            h = x_v[pl.ds(rw, m), :].astype(F32) + jnp.dot(o[m * u:m * (u + 1)].astype(BF), wo_v[...], preferred_element_type=F32)
            hs.append(h)
            hns.append(_ln(h).astype(BF))
        return jnp.concatenate(hs, axis=0), jnp.concatenate(hns, axis=0)

    def ffn(h, hn, row, splits):
        acc = h
        nc = F // FC
        for c in range(nc):
            gate = jnp.dot(hn, w1_v[:, pl.ds(FC * c, FC)], preferred_element_type=F32)
            up = jnp.dot(hn, w3_v[:, pl.ds(FC * c, FC)], preferred_element_type=F32)
            hg = 0.5 * gate
            act = (hg + hg * jnp.tanh(hg)) * up
            if c + 1 < nc:
                acc = acc + jnp.dot(act.astype(BF), w2_v[pl.ds(FC * c, FC), :], preferred_element_type=F32)
        r0 = 0
        for n, cols in splits:
            rw = pl.multiple_of(row + r0, 64)
            c0 = 0
            a = act[r0:r0 + n].astype(BF)
            for nc in cols:
                res = acc[r0:r0 + n, c0:c0 + nc] + jnp.dot(a, w2_v[pl.ds(F - FC, FC), pl.ds(c0, nc)],
                                                           preferred_element_type=F32)
                out_v[pl.ds(rw, n), pl.ds(c0, nc)] = res.astype(BF)
                ocopy(rw, n, c0, nc).start()
                c0 += nc
            r0 += n

    nsub = TB // SB
    splits = [((SB, (D,)),)] * (nsub - 1) + [OSPLIT]

    def body_b(j, carry):
        rows = [pl.multiple_of(j * TB + s * SB, SB) for s in range(nsub)]
        qs, os_, hs, nf = [], [], [], 0
        for o in ORB:
            if o == "Q":
                qs.append(feats(0, rows[len(qs)], SB))
            elif o == "A":
                os_.append(attn(qs[len(os_)]))
            elif o == "W":
                hs.append(oproj(rows[len(hs)], os_[len(hs)]))
            else:
                ffn(*hs[nf], rows[nf], splits[nf])
                nf += 1
        assert nf == nsub
        return carry

    with jax.named_scope("phaseB"):
        lax.fori_loop(0, NB, body_b, 0)

    with jax.named_scope("tail"):
        for j in range(NB):
            r0 = j * TB
            for sp in splits:
                for n, cols in sp:
                    c0 = 0
                    for nc in cols:
                        ocopy(r0, n, c0, nc).wait()
                        c0 += nc
                    r0 += n


def _full(c0, c1):
    return [(c,) for c in range(c0, c1)]


_PRO = [([("x", 3)], 2, ["T"]),
        ([("k", 1)], 1, [("N", 0, 3, 0, 1, 4), "T"]),
        ([("k", 2)], 0, [("N", 0, 3, 1, 2, 2), "T"]),
        ([("k", 2), ("x", 2)], 2, [("N", 0, 3, 3, 2, 2), "T", (3,), (4, 1, 0, 2)]),
        ([("x", 6), ("p", 0)], 0, [(4, 1, 2, 3), (5,), ("X", 0), (6,), ("X", 1), (7,), "B", ("X", 2)] + _full(8, 11)),
        ([("w", 0), ("x", 5)], 0, ["k0257", "q0257", "k13", (11,), (12,), "k4", (13,), "k6", (14,), (15,)]
         + list("KKAAKKAA") + ["q1346"])]


def build(A_x, A_wqkv, A_w_phi, A_wo, B_x, B_w1, B_w3, B_w2, TA=512, TB=512, SB=256, FC=512,
          ORB="QQAAWWFF", WP=4, PRO=_PRO, OSPLIT=((128, (D,)), (64, (D,)), (64, (384, 128, 128)))):
    x2 = A_x.reshape(S, D)
    wphi_t = A_w_phi.transpose(1, 2, 0)
    any_spec = pl.BlockSpec(memory_space=pl.ANY)
    out = pl.pallas_call(
        functools.partial(_kernel, TA=TA, TB=TB, SB=SB, FC=FC, OSPLIT=OSPLIT, ORB=ORB, WP=WP, PRO=PRO),
        in_specs=[any_spec] * 7,
        out_specs=any_spec,
        out_shape=jax.ShapeDtypeStruct((S, D), BF),
        scratch_shapes=[
            pltpu.VMEM((S, D), BF),
            pltpu.VMEM((S, D), BF),
            pltpu.VMEM((S, D), BF),
            pltpu.VMEM((NG, 64, S), BF),
            pltpu.VMEM((DH, DH, H), BF),
            pltpu.VMEM((D, 3 * D), BF),
            pltpu.VMEM((D, D), BF),
            pltpu.VMEM((D, F), BF),
            pltpu.VMEM((D, F), BF),
            pltpu.VMEM((F, D), BF),
            pltpu.VMEM((3 * D, D), BF),
            pltpu.VMEM((8, PR, 128), F32),
            pltpu.VMEM((5, 128, 128), F32),
            pltpu.VMEM((D, 128), F32),
            pltpu.VMEM((NG - 1, 64, 128), BF),
            pltpu.VMEM((48, 2 * PR), BF),
            pltpu.VMEM((3, 64, 128), jnp.int32),
            pltpu.VMEM((D, 128), F32),
            pltpu.VMEM((384, D), F32),
            pltpu.VMEM((8, 2 * PR, 128), BF),
            pltpu.SemaphoreType.DMA((len(PRO) - 1,)),
        ],
        compiler_params=pltpu.CompilerParams(
            vmem_limit_bytes=100 * 1024 * 1024,
            disable_bounds_checks=True,
        ),
    )(x2, A_wqkv, wphi_t, A_wo, B_w1, B_w3, B_w2)
    return out.reshape(1, S, D)


@jax.jit
def pallas_sequential_preLN__linear_kernel_hedgehog__glu_gated_swiglu__prompt_kernel(
        A_x, A_wqkv, A_w_phi, A_wo, B_x, B_w1, B_w3, B_w2):
    return build(A_x, A_wqkv, A_w_phi, A_wo, B_x, B_w1, B_w3, B_w2)
```

```python
import functools
import math
import jax
import jax.numpy as jnp
from jax import lax
import jax.experimental.pallas as pl
import jax.experimental.pallas.tpu as pltpu

S, D, H, DH, F = 2048, 640, 32, 20, 1536
PR = 2 * DH
NS = 5
NG = 2 * NS + 1
SEXT = ((2, 3, 4), (5, 6, 7), (8, 9, 10), (11, 12, 13), (0, 1, 14))
MIDS = tuple(m for _, m, _ in SEXT)
FC0 = (0, 80, 128, 240, 320, 384, 480, 512)
NT_DIMS = (((1,), (1,)), ((), ()))
BF = jnp.bfloat16
F32 = jnp.float32
EPS = 1e-5
LOG2E = 1.4426950408889634


def _rcp(x):
    r = pl.reciprocal(x, approx=True)
    return r * (2.0 - x * r)


def _ln(x):
    m = jnp.mean(x, axis=-1, keepdims=True)
    xc = x - m
    v = jnp.mean(xc * xc, axis=-1, keepdims=True)
    return xc * lax.rsqrt(v + EPS)


def _red(x3, op):
    r = op(op(op(x3[0], x3[1]), op(x3[2], x3[3])), x3[4])
    r = op(r, pltpu.roll(r, 2, 0))
    r = op(r, pltpu.roll(r, 4, 0))
    return r


def _feat(p, T):
    p3 = p.reshape(5, 8, T)
    mx = _red(p3, jnp.maximum)
    mn = _red(p3, jnp.minimum)
    ep = jnp.exp2(p3 - mx[None])
    en = jnp.exp2(mn[None] - p3)
    rp = _rcp(_red(ep, jnp.add))
    rn = _rcp(_red(en, jnp.add))
    phi = jnp.concatenate([ep * rp[None], en * rn[None]], axis=0)
    return phi.reshape(2 * PR, T)


def _feat_split(p, T):
    even = lax.broadcasted_iota(jnp.int32, (8, T), 0) % 2 == 0

    def red(x3, op):
        m0, m1 = op(x3[0], x3[1]), op(x3[2], x3[3])
        r = op(op(jnp.where(even, m0, m1), pltpu.roll(jnp.where(even, m1, m0), 1, 0)), x3[4])
        r = op(r, pltpu.roll(r, 2, 0))
        return op(r, pltpu.roll(r, 4, 0))

    def spread(r):
        rs = pltpu.roll(r, 1, 0)
        r0, r1 = jnp.where(even, r, rs), jnp.where(even, rs, r)
        return jnp.stack([r0, r0, r1, r1, r], axis=0)

    p3 = p.reshape(5, 8, T)
    ep = jnp.exp2(p3 - spread(red(p3, jnp.maximum)))
    en = jnp.exp2(spread(red(p3, jnp.minimum)) - p3)
    ep = ep * spread(_rcp(red(ep, jnp.add)))
    en = en * spread(_rcp(red(en, jnp.add)))
    out = [jnp.concatenate([ep[i:j], en[i:j]], axis=0) for i, j in ((0, 2), (2, 4), (4, 5))]
    return [o.reshape(-1, T) for o in out]


def _kernel(x_hbm, wqkv_hbm, wphi_hbm, wo_hbm, w1_hbm, w3_hbm, w2_hbm, out_hbm,
            x_v, out_v, xn_v, vt_v, wphi_v, wqkv_v, wo_v, w1_v, w3_v, w2_v, wt_v, wp_v, wn_v, y_v, kvb_v, kvl_v, mk_v, va_v, vn_v, as_v,
            sems, *, TA, TB, SB, FC, OSPLIT, ORB, WP, PRO):
    NB = S // TB

    def wcopy(c0, n, sem):
        return pltpu.make_async_copy(wqkv_hbm.at[:, pl.ds(c0, n)], wqkv_v.at[:, pl.ds(c0, n)], sems.at[sem])

    def xcopy(r0, r1, sem):
        return pltpu.make_async_copy(x_hbm.at[pl.ds(r0, r1 - r0)], x_v.at[pl.ds(r0, r1 - r0)], sems.at[sem])

    def ocopy(r, n, c0=0, nc=D):
        return pltpu.make_async_copy(out_v.at[pl.ds(r, n), pl.ds(c0, nc)], out_hbm.at[pl.ds(r, n), pl.ds(c0, nc)],
                                     sems.at[1])

    def vcopy(r0, n, sem):
        return pltpu.make_async_copy(wqkv_hbm.at[pl.ds(r0, n), pl.ds(2 * D, D)],
                                     wqkv_v.at[pl.ds(r0, n), pl.ds(2 * D, D)], sems.at[sem])

    groups, nx, nk = [], 0, 0
    for g, (pieces, _, _) in enumerate(PRO):
        cps, sem = [], g % (len(PRO) - 1)
        for kind, n in pieces:
            if kind == "x":
                cps.append(xcopy(128 * nx, 128 * (nx + n), sem))
                nx += n
            elif kind == "k":
                cps.append(vcopy(128 * nk, 128 * n, sem))
                nk += n
            elif kind == "p":
                cps.append(pltpu.make_async_copy(wphi_hbm, wphi_v, sems.at[sem]))
            else:
                cps.append(wcopy(0, 2 * D, sem))
        groups.append(cps)
    assert nk == 5 and 128 * nx == S
    cp_wo = pltpu.make_async_copy(wo_hbm, wo_v, sems.at[1])
    cp_w1 = pltpu.make_async_copy(w1_hbm, w1_v, sems.at[1])
    cp_w3 = pltpu.make_async_copy(w3_hbm, w3_v, sems.at[1])
    cp_w2 = pltpu.make_async_copy(w2_hbm, w2_v, sems.at[1])

    def wstart():
        cp_wo.start(); cp_w1.start(); cp_w3.start(); cp_w2.start()

    def dot2(w, xn, ms=None):
        tiles = (xn.shape[0] // 128) * (xn.shape[1] // 128)
        ns = 4 // math.gcd(4, tiles)
        ms = ms or [w.shape[0] // ns] * ns
        return jnp.concatenate([lax.dot_general(w[sum(ms[:u]):sum(ms[:u + 1])], xn, NT_DIMS,
                                                preferred_element_type=F32) for u in range(len(ms))], axis=0)

    def vstore(pv, c0, n):
        low = lax.broadcasted_iota(jnp.int32, (8, n), 0) < 4
        for q, (a, m, c) in enumerate(SEXT):
            r = PR * m
            mid = pv[r + 16:r + 24]
            vt_v[2 * q, :, pl.ds(c0, n)] = jnp.concatenate(
                [pv[PR * a:PR * (a + 1)], pv[r:r + 16], jnp.where(low, mid, 1.0)], axis=0).astype(BF)
            vt_v[2 * q + 1, :, pl.ds(c0, n)] = jnp.concatenate(
                [jnp.where(low, 1.0, mid), pv[r + 24:r + PR], pv[PR * c:PR * (c + 1)]], axis=0).astype(BF)
        vt_v[NG - 1, pl.ds(0, 48), pl.ds(c0, n)] = jnp.concatenate(
            [pv[D - PR:], jnp.ones((8, n), F32)], axis=0).astype(BF)

    def transpose_v(k):
        wt_v[pl.ds(2 * D, D), pl.ds(128 * k, 128)] = (
            wqkv_v[pl.ds(128 * k, 128), pl.ds(2 * D, D)].astype(F32).T.astype(BF))

    def vdot(c, nt, k, nk):
        return dot2(wt_v[pl.ds(2 * D, D), pl.ds(128 * k, 128 * nk)],
                    xn_v[pl.ds(128 * c, 128 * nt), pl.ds(128 * k, 128 * nk)])

    def ndot(c, nt, k, nk, ns):
        m = 128 * nt // ns
        return jnp.concatenate([jnp.dot(xn_v[pl.ds(128 * c + m * u, m), pl.ds(128 * k, 128 * nk)],
                                        wqkv_v[pl.ds(128 * k, 128 * nk), pl.ds(2 * D, D)],
                                        preferred_element_type=F32) for u in range(ns)], axis=0)

    def fold(As, s, gs):
        for g in gs:
            res = dot2(As[g][...], wqkv_v[:, pl.ds(D * s + FC0[g], 128)], [2 * PR])
            wt_v[pl.ds(D * s + 2 * PR * g, 2 * PR), :] = (res * LOG2E).astype(BF)

    def feats(s, row, n):
        pk = dot2(wt_v[pl.ds(D * s, D), :], xn_v[pl.ds(row, n), :])
        out = []
        for a, m, c in SEXT:
            fa = _feat(pk[PR * a:PR * (a + 1)], n)
            f0, f1, fm = _feat_split(pk[PR * m:PR * (m + 1)], n)
            fc = _feat(pk[PR * c:PR * (c + 1)], n)
            out += [jnp.concatenate([fa, f0, fm], axis=0).astype(BF), jnp.concatenate([fc, f1, fm], axis=0).astype(BF)]
        return out + [_feat(pk[D - PR:], n).astype(BF)]

    def astep(kvs, b, phiks):
        out = []
        for g in range(NG):
            m = 64 if g < NG - 1 else 48
            kv = lax.dot_general(vt_v[g, pl.ds(0, m), pl.ds(TA * b, TA)], phiks[g], NT_DIMS,
                                 preferred_element_type=F32)
            out.append(kv if kvs is None else kv + kvs[g])
        return out

    def lnt(c, n=128):
        xn_v[pl.ds(128 * c, n), :] = _ln(x_v[pl.ds(128 * c, n), :].astype(F32)).astype(BF)

    with jax.named_scope("prologue"):
        for cps in groups[:-1]:
            for cp in cps:
                cp.start()

        c8 = lax.broadcasted_iota(jnp.int32, (8, 128), 1)
        r8 = lax.broadcasted_iota(jnp.int32, (8, 128), 0)
        wn_v[...] = jnp.zeros(wn_v.shape, F32)

        rr = lax.broadcasted_iota(jnp.int32, (64, 128), 0)
        cc = lax.broadcasted_iota(jnp.int32, (64, 128), 1)
        par = cc % 2
        for e in range(2):
            head_c = jnp.where(cc < 2 * PR, par, jnp.where((cc < 112) | (par == e), 2, 3))
            if e == 0:
                head_r = jnp.where(rr < 60, rr // DH, jnp.minimum(rr - 60, 2))
            else:
                head_r = (jnp.where(rr < 4, jnp.minimum(rr, 2), (rr - 4) // DH) + 2) % 3
            mk_v[e] = head_r - head_c
        mk_v[2] = jnp.where(rr < PR, rr // DH, (rr - PR) // 4) - par

        def cmat():
            w = wphi_v[...].astype(F32)
            for g in range(5):
                wn_v[g, pl.ds(0, DH), :] = jnp.concatenate([w[4 * g + l] for l in range(4)], axis=1)
                wg = wn_v[g].T
                for l in range(4):
                    y_v[pl.ds(4 * g + l, H, stride=DH), :] = wg[H * l:H * (l + 1)]
            return y_v[...].T[:24]

        def abuild(C):
            B1 = C.reshape(3, 8, D)
            As = []
            for g, c0 in enumerate(FC0):
                b1 = B1[:, :, c0:c0 + 128]
                b20 = b1.reshape(24, 128)[:DH]
                wp_v[g, pl.ds(0, DH, stride=2), :] = b20
                wp_v[g, pl.ds(1, DH, stride=2), :] = b20
                b2 = wp_v[g].reshape(5, 8, 128)
                ch = (c8 + c0) // DH
                hp = ch - r8 % 2
                rows = []
                for p in (2 * g, 2 * g + 1):
                    if p in MIDS:
                        rows += [jnp.where((ch == h)[None], b1[:2], 0.0) for h in (2 * p, 2 * p + 1)]
                        rows.append(jnp.where((hp == 2 * p)[None], b2[4:], 0.0))
                    else:
                        rows.append(jnp.where((hp == 2 * p)[None], b2, 0.0))
                As.append(jnp.concatenate(rows, axis=0).reshape(2 * PR, 128).astype(BF))
            return As

        done = [0] * (S // 128)
        nl = nt_ = nk = na = 0
        kvs, phiks, As = None, {}, None
        for g, (pieces, lns, units) in enumerate(PRO):
            with jax.named_scope(f"w_{g}"):
                for cp in groups[g]:
                    cp.wait()
            if g == 0:
                for cp in groups[-1]:
                    cp.start()
            if g == len(PRO) - 1:
                wstart()
            acc, nl0 = {}, nl
            news = sum(n for kind, n in pieces if kind == "k")
            for u in units:
                if u == "T":
                    for k in range(nt_, nt_ + news):
                        transpose_v(k)
                    nt_ += news
                    for c in range(nl, nl0 + lns):
                        lnt(c)
                    nl = max(nl, nl0 + lns)
                elif u == "B":
                    for t, a in enumerate(abuild(cmat())):
                        as_v[t] = a
                    As = [as_v.at[t] for t in range(8)]
                elif u[0] in ("k", "q"):
                    fold(As, 1 if u[0] == "k" else 0, [int(g) for g in u[1:]])
                elif u == "K":
                    phiks[nk] = feats(1, TA * nk, TA)
                    nk += 1
                elif u == "A":
                    assert all(d == 5 for d in done[4 * na:4 * na + 4])
                    kvs = astep(kvs, na, phiks.pop(na))
                    na += 1
                elif u[0] == "N":
                    _, c0, nt, k, n, ns = u
                    for c in range(nl, c0 + nt):
                        lnt(c)
                    nl = max(nl, c0 + nt)
                    r = ndot(c0, nt, k, n, ns)
                    assert all(d == k for d in done[c0:c0 + nt])
                    if k:
                        r = r + vn_v[pl.ds(128 * c0, 128 * nt), :]
                    vn_v[pl.ds(128 * c0, 128 * nt), :] = r
                    done[c0:c0 + nt] = [k + n if k + n < 5 else -1] * nt
                elif u[0] == "X":
                    assert done[u[1]] == -1
                    vstore(vn_v[pl.ds(128 * u[1], 128), :].T, 128 * u[1], 128)
                    done[u[1]] = 5
                else:
                    c0, nt, k, n = u if len(u) == 4 else (u[0], 1, 0, 5)
                    for c in range(nl, c0 + nt):
                        lnt(c)
                    nl = max(nl, c0 + nt)
                    r = vdot(c0, nt, k, n)
                    for c in range(c0, c0 + nt):
                        rc = r[:, 128 * (c - c0):128 * (c - c0 + 1)]
                        if done[c]:
                            rc = rc + (acc[c] if c in acc else va_v[...])
                        done[c] += n
                        acc[c] = rc
                        if done[c] == 5:
                            vstore(acc.pop(c), 128 * c, 128)
            assert len(acc) <= 1
            for rc in acc.values():
                va_v[...] = rc
        assert nl == S // 128 and nk == na == S // TA
        for g in range(NG - 1):
            kvb_v[g] = jnp.where(mk_v[g % 2] == 0, kvs[g], 0.0).astype(BF)
        kvl_v[...] = jnp.where(mk_v[2, pl.ds(0, 48), pl.ds(0, 2 * PR)] == 0, kvs[NG - 1], 0.0).astype(BF)
        with jax.named_scope("w_w"):
            cp_wo.wait(); cp_w1.wait(); cp_w3.wait(); cp_w2.wait()

    def attn(phiq):
        low = lax.broadcasted_iota(jnp.int32, (8, SB), 0) < 4
        ots = []
        for q in range(NS):
            n1 = jnp.dot(kvb_v[2 * q], phiq[2 * q], preferred_element_type=F32)
            n2 = jnp.dot(kvb_v[2 * q + 1], phiq[2 * q + 1], preferred_element_type=F32)
            r = _rcp(jnp.where(low, n2[:8], n1[56:]) + 1e-6)
            ra, rb, rc, rd, re, rf = [jnp.broadcast_to(r[k:k + 1], (8, SB)) for k in (4, 5, 6, 0, 1, 2)]
            num = jnp.concatenate([n1[:56], jnp.where(low, n1[56:], n2[:8]), n2[8:]], axis=0)
            scale = jnp.concatenate([ra, ra, jnp.where(low, ra, rb), rb, rb, rc, rc, jnp.where(low, rc, rd),
                                     rd, rd, re, re, jnp.where(low, re, rf), rf, rf], axis=0)
            ots.append(num * scale)
        ots = [ots[-1][:2 * PR]] + ots[:-1] + [ots[-1][2 * PR:]]
        nd = jnp.dot(kvl_v[...], phiq[NG - 1], preferred_element_type=F32)
        r = _rcp(nd[PR:PR + 8] + 1e-6)
        rs = pltpu.roll(r, 4, 0)
        ra = jnp.where(low, r, rs)
        rb = jnp.where(low, rs, r)
        ots.append(nd[:PR] * jnp.concatenate([ra, ra, r, rb, rb], axis=0))
        return jnp.concatenate(ots, axis=0).T

    def oproj(row, o):
        hs, hns = [], []
        m = SB // WP
        for u in range(WP):
            rw = pl.multiple_of(row + m * u, m)
            h = x_v[pl.ds(rw, m), :].astype(F32) + jnp.dot(o[m * u:m * (u + 1)].astype(BF), wo_v[...], preferred_element_type=F32)
            hs.append(h)
            hns.append(_ln(h).astype(BF))
        return jnp.concatenate(hs, axis=0), jnp.concatenate(hns, axis=0)

    def ffn(h, hn, row, splits):
        acc = h
        nc = F // FC
        for c in range(nc):
            gate = jnp.dot(hn, w1_v[:, pl.ds(FC * c, FC)], preferred_element_type=F32)
            up = jnp.dot(hn, w3_v[:, pl.ds(FC * c, FC)], preferred_element_type=F32)
            hg = 0.5 * gate
            act = (hg + hg * jnp.tanh(hg)) * up
            if c + 1 < nc:
                acc = acc + jnp.dot(act.astype(BF), w2_v[pl.ds(FC * c, FC), :], preferred_element_type=F32)
        r0 = 0
        for n, cols in splits:
            rw = pl.multiple_of(row + r0, 64)
            c0 = 0
            a = act[r0:r0 + n].astype(BF)
            for nc in cols:
                res = acc[r0:r0 + n, c0:c0 + nc] + jnp.dot(a, w2_v[pl.ds(F - FC, FC), pl.ds(c0, nc)],
                                                           preferred_element_type=F32)
                out_v[pl.ds(rw, n), pl.ds(c0, nc)] = res.astype(BF)
                ocopy(rw, n, c0, nc).start()
                c0 += nc
            r0 += n

    nsub = TB // SB
    splits = [((SB, (D,)),)] * (nsub - 1) + [OSPLIT]

    def body_b(j, carry):
        rows = [pl.multiple_of(j * TB + s * SB, SB) for s in range(nsub)]
        qs, os_, hs, nf = [], [], [], 0
        for o in ORB:
            if o == "Q":
                qs.append(feats(0, rows[len(qs)], SB))
            elif o == "A":
                os_.append(attn(qs[len(os_)]))
            elif o == "W":
                hs.append(oproj(rows[len(hs)], os_[len(hs)]))
            else:
                ffn(*hs[nf], rows[nf], splits[nf])
                nf += 1
        assert nf == nsub
        return carry

    with jax.named_scope("phaseB"):
        lax.fori_loop(0, NB, body_b, 0)

    with jax.named_scope("tail"):
        for j in range(NB):
            r0 = j * TB
            for sp in splits:
                for n, cols in sp:
                    c0 = 0
                    for nc in cols:
                        ocopy(r0, n, c0, nc).wait()
                        c0 += nc
                    r0 += n


_PRO = [([("x", 3)], 3, ["T"]),
        ([("k", 1), ("x", 1)], 1, [("N", 0, 4, 0, 1, 4), "T"]),
        ([("k", 2)], 0, [("N", 0, 4, 1, 2, 2), "T"]),
        ([("k", 2), ("x", 1)], 1, [("N", 0, 4, 3, 2, 2), "T", (4, 1, 0, 2)]),
        ([("x", 6), ("p", 0)], 0, [(4, 1, 2, 3), (5,), ("X", 0), (6,), ("X", 1), (7,), "B", ("X", 2), (8,), ("X", 3),
                                   (9,), (10,)]),
        ([("w", 0), ("x", 5)], 0, ["k0257", "q0257", "k13", (11,), (12,), "k4", (13,), "k6", (14,), (15,)]
         + list("KKAAKKAA") + ["q1346"])]


def build(A_x, A_wqkv, A_w_phi, A_wo, B_x, B_w1, B_w3, B_w2, TA=512, TB=512, SB=256, FC=512,
          ORB="QQAAWWFF", WP=4, PRO=_PRO, OSPLIT=((128, (D,)), (64, (D,)), (64, (384, 128, 128)))):
    x2 = A_x.reshape(S, D)
    wphi_t = A_w_phi.transpose(1, 2, 0)
    any_spec = pl.BlockSpec(memory_space=pl.ANY)
    out = pl.pallas_call(
        functools.partial(_kernel, TA=TA, TB=TB, SB=SB, FC=FC, OSPLIT=OSPLIT, ORB=ORB, WP=WP, PRO=PRO),
        in_specs=[any_spec] * 7,
        out_specs=any_spec,
        out_shape=jax.ShapeDtypeStruct((S, D), BF),
        scratch_shapes=[
            pltpu.VMEM((S, D), BF),
            pltpu.VMEM((S, D), BF),
            pltpu.VMEM((S, D), BF),
            pltpu.VMEM((NG, 64, S), BF),
            pltpu.VMEM((DH, DH, H), BF),
            pltpu.VMEM((D, 3 * D), BF),
            pltpu.VMEM((D, D), BF),
            pltpu.VMEM((D, F), BF),
            pltpu.VMEM((D, F), BF),
            pltpu.VMEM((F, D), BF),
            pltpu.VMEM((3 * D, D), BF),
            pltpu.VMEM((8, PR, 128), F32),
            pltpu.VMEM((5, 128, 128), F32),
            pltpu.VMEM((D, 128), F32),
            pltpu.VMEM((NG - 1, 64, 128), BF),
            pltpu.VMEM((48, 2 * PR), BF),
            pltpu.VMEM((3, 64, 128), jnp.int32),
            pltpu.VMEM((D, 128), F32),
            pltpu.VMEM((512, D), F32),
            pltpu.VMEM((8, 2 * PR, 128), BF),
            pltpu.SemaphoreType.DMA((len(PRO) - 1,)),
        ],
        compiler_params=pltpu.CompilerParams(
            vmem_limit_bytes=100 * 1024 * 1024,
            disable_bounds_checks=True,
        ),
    )(x2, A_wqkv, wphi_t, A_wo, B_w1, B_w3, B_w2)
    return out.reshape(1, S, D)


@jax.jit
def pallas_sequential_preLN__linear_kernel_hedgehog__glu_gated_swiglu__prompt_kernel(
        A_x, A_wqkv, A_w_phi, A_wo, B_x, B_w1, B_w3, B_w2):
    return build(A_x, A_wqkv, A_w_phi, A_wo, B_x, B_w1, B_w3, B_w2)
```
